```python
import jax
import jax.numpy as jnp

def _softmax(x, axis=-1):
    return jax.nn.softmax(x, axis=axis)

def _gelu(x):
    return jax.nn.gelu(x, approximate=True)

def _silu(x):
    return jax.nn.silu(x)

def _sigmoid(x):
    return jax.nn.sigmoid(x)

def _layernorm(x, axis=-1, eps=1e-05):
    m = jnp.mean(x, axis=axis, keepdims=True)
    v = jnp.var(x, axis=axis, keepdims=True)
    return (x - m) / jnp.sqrt(v + eps)

def _scatter_add(tgt, idx, src, axis=0):
    return tgt.at[idx].add(src)

def _segment_sum(src, seg, n):
    return jax.ops.segment_sum(src, seg, n)

class _Rng:

    def __init__(self, key):
        self._k = key

    def _next(self):
        self._k, sub = jax.random.split(self._k)
        return sub

    def normal(self, shape):
        return jax.random.normal(self._next(), shape, dtype=jnp.bfloat16)

    def randint(self, lo, hi, shape):
        return jax.random.randint(self._next(), shape, lo, hi, dtype=jnp.int32)

    def uniform(self, shape, lo=0.0, hi=1.0):
        return jax.random.uniform(self._next(), shape, jnp.bfloat16, lo, hi)

    def permutation(self, n):
        return jax.random.permutation(self._next(), n)
kernel_name = 'adaLN_cond__mha_block_cached__moe_arch_mod__prompt'

def setup_inputs():
    _rng = _Rng(jax.random.key(int.from_bytes(__import__("os").urandom(4), "little")))
    _w = lambda a: (lambda t: t.astype(jnp.bfloat16) if jnp.issubdtype(t.dtype, jnp.floating) else t)(jnp.asarray(a))

    def _A_setup():
        B, Sq, D = (1, 2048, 1024)
        H, Sk, Dh = (32, 2048, 128)
        return {'x': _w((lambda *s: _rng.normal(s) * 0.05)(B, Sq, D)), 'k_cache': _w((lambda *s: _rng.normal(s) * 0.05)(B, H, Sk, Dh)), 'v_cache': _w((lambda *s: _rng.normal(s) * 0.05)(B, H, Sk, Dh)), 'wq': _w((lambda *s: _rng.normal(s) * 0.05)(D, H * Dh) * D ** (-0.5)), 'wo': _w((lambda *s: _rng.normal(s) * 0.05)(H * Dh, D) * (H * Dh) ** (-0.5))}
    _A_in = _A_setup()

    def _B_setup():
        B, S, D, F, C = (1, 2048, 1024, 3584, 2)
        return {'x': _w((lambda *s: _rng.normal(s) * 0.05)(B, S, D)), 'w_r': _w((lambda *s: _rng.normal(s) * 0.05)(D)), 'w_gate': _w((lambda *s: _rng.normal(s) * 0.05)(D, F)), 'w_up': _w((lambda *s: _rng.normal(s) * 0.05)(D, F)), 'w_down': _w((lambda *s: _rng.normal(s) * 0.05)(F, D))}
    _B_in = _B_setup()
    return {'A_x': _A_in['x'], 'A_k_cache': _A_in['k_cache'], 'A_v_cache': _A_in['v_cache'], 'A_wq': _A_in['wq'], 'A_wo': _A_in['wo'], 'B_x': _B_in['x'], 'B_w_r': _B_in['w_r'], 'B_w_gate': _B_in['w_gate'], 'B_w_up': _B_in['w_up'], 'B_w_down': _B_in['w_down'], 'c': _w((lambda *s: _rng.normal(s) * 0.05)(1, 1024)), 'w_mod': _w((lambda *s: _rng.normal(s) * 0.05)(1024, 6 * 1024) * 1024 ** (-0.5))}

def reference(A_x, A_k_cache, A_v_cache, A_wq, A_wo, B_x, B_w_r, B_w_gate, B_w_up, B_w_down, c, w_mod):

    def _A_ref(x, k_cache, v_cache, wq, wo):
        B, Sq, D = x.shape
        H, Dh = (32, 128)
        q = (lambda x, *d: x.transpose(*d))((x @ wq).reshape(B, Sq, H, Dh), 0, 2, 1, 3)
        scores = jnp.einsum('bhqd,bhkd->bhqk', q, k_cache) * Dh ** (-0.5)
        p = _softmax(scores, axis=-1)
        o = jnp.einsum('bhqk,bhkd->bhqd', p, v_cache)
        return (lambda x, *d: x.transpose(*d))(o, 0, 2, 1, 3).reshape(B, Sq, H * Dh) @ wo

    def _B_ref(x, w_r, w_gate, w_up, w_down):
        B, S, D = x.shape
        C = 2
        r = x @ w_r
        idx = jnp.argsort(-r, axis=-1)[:, :C]
        idx_e = jnp.repeat(idx.reshape(B, C, 1), D, axis=2)
        x_sel = jnp.take_along_axis(x, idx_e, axis=1)
        g = _silu(x_sel @ w_gate)
        u = x_sel @ w_up
        y = g * u @ w_down
        r_sel = _sigmoid(jnp.take_along_axis(r, idx, axis=1))
        y = y * r_sel.reshape(B, C, 1)
        b_off = (jnp.arange(B) * S).reshape(B, 1)
        flat_idx = (idx + b_off).reshape(B * C)
        zero = (x * 0.0).reshape(B * S, D)
        upd = _scatter_add(zero, flat_idx, y.reshape(B * C, D), axis=0)
        return x + upd.reshape(B, S, D)
    x = A_x
    mod = (_silu(c) @ w_mod).reshape(c.shape[0], 6, 1, -1)
    sa, ca, ga, sb, cb, gb = (mod[:, 0].copy(), mod[:, 1].copy(), mod[:, 2].copy(), mod[:, 3].copy(), mod[:, 4].copy(), mod[:, 5].copy())
    h = _layernorm(x, axis=-1) * (1 + ca) + sa
    x = x + ga * _A_ref(h, A_k_cache, A_v_cache, A_wq, A_wo)
    h = _layernorm(x, axis=-1) * (1 + cb) + sb
    x = x + gb * _B_ref(h, B_w_r, B_w_gate, B_w_up, B_w_down)
    return x
```

```python
import functools
import math

import jax
import jax.numpy as jnp
from jax import lax
from jax.experimental import pallas as pl
from jax.experimental.pallas import tpu as pltpu

F32 = jnp.float32
BF16 = jnp.bfloat16

S = 2048
D = 1024
H = 32
DH = 128
FF = 3584
EPS = 1e-5
QSCALE = (DH ** -0.5) * math.log2(math.e)

G = 4
SUB = 512
N0 = 512
XC = 256
NX = S // XC
MC = 512
NT = (((1,), (1,)), ((), ()))

_names = (["c", "wr", "wq0", "wq1", "wg", "wu", "wd", "wo", "wm2", "f0", "f1"]
          + ["wm%d" % i for i in range(4, 8)] + ["x%d" % i for i in range(NX)]
          + ["k0", "k1", "v0", "v1"] + ["o%d" % i for i in range(S // MC)])
_SEM = {n: i for i, n in enumerate(_names)}


def _attn(q, k, v):
    s = lax.dot_general(q, k, NT, preferred_element_type=F32)
    m = jnp.max(s, axis=1, keepdims=True)
    p = jnp.exp2(s - m)
    grp = 4
    acc = None
    tiles = []
    for g in range(S // (128 * grp)):
        ts = [p[:, (g * grp + j) * 128:(g * grp + j + 1) * 128] for j in range(grp)]
        t = (ts[0] + ts[1]) + (ts[2] + ts[3])
        acc = t if acc is None else acc + t
        tiles += ts[:-1] + [jnp.minimum(ts[-1], acc)]
    l = jnp.sum(acc, axis=1, keepdims=True)
    o = jnp.dot(jnp.concatenate(tiles, axis=1).astype(BF16), v, preferred_element_type=F32)
    return (o * pl.reciprocal(l, approx=True)).astype(BF16)


def _kernel(x_hbm, k_hbm, v_hbm, wq_hbm, wo_hbm, wr_hbm, wg_hbm, wu_hbm, wd_hbm,
            c_hbm, wm_hbm, out_hbm,
            x_v, h_v, wq_v, q_v, o_v, k_v, v_v, wo_v, out_v, wr_v, wg_v, wu_v, wd_v, c_v,
            wm_v, mod_v, r_v, fix_v, sems):

    def cp(name, src, dst):
        return pltpu.make_async_copy(src, dst, sems.at[_SEM[name]])

    c_cp = cp("c", c_hbm, c_v)
    wm_cps = [cp("wm%d" % (4 + i), wm_hbm.at[:, pl.ds(i * 512, 512)], wm_v.at[:, pl.ds(i * 512, 512)])
              for i in range(4)]
    wm2_cp = cp("wm2", wm_hbm.at[:, pl.ds(2 * D, 4 * D)], wm_v.at[:, pl.ds(2 * D, 4 * D)])
    x_cps = [cp("x%d" % i, x_hbm.at[pl.ds(i * XC, XC), :], x_v.at[pl.ds(i * XC, XC), :])
             for i in range(NX)]
    wq0_cp = cp("wq0", wq_hbm.at[:, pl.ds(0, N0)], wq_v.at[:, pl.ds(0, N0)])
    wq1_cp = cp("wq1", wq_hbm.at[:, pl.ds(N0, H * DH - N0)], wq_v.at[:, pl.ds(N0, H * DH - N0)])
    wo_cp = cp("wo", wo_hbm, wo_v)
    wr_cp = cp("wr", wr_hbm, wr_v)
    wg_cp = cp("wg", wg_hbm, wg_v)
    wu_cp = cp("wu", wu_hbm, wu_v)
    wd_cp = cp("wd", wd_hbm, wd_v)

    def kv_cps(grp, slot):
        heads = pl.ds(grp * G, G)
        return (pltpu.make_async_copy(k_hbm.at[heads], k_v.at[slot], sems.at[_SEM["k0"] + slot]),
                pltpu.make_async_copy(v_hbm.at[heads], v_v.at[slot], sems.at[_SEM["v0"] + slot]))

    c_cp.start()
    for w in wm_cps:
        w.start()
    x_cps[0].start()
    wq0_cp.start()
    for xc in x_cps[1:]:
        xc.start()
    wq1_cp.start()

    c_cp.wait()
    cf = c_v[...].astype(F32)
    sc = jnp.broadcast_to(cf * jax.nn.sigmoid(cf), (16, D)).astype(BF16)
    for i in range(4):
        wm_cps[i].wait()
        cols = pl.ds(i * 512, 512)
        mod_v[:, cols] = jnp.dot(sc, wm_v[:, cols], preferred_element_type=F32)[:8]

    def store_q(q, rows, head0):
        q = (q * QSCALE).astype(BF16)
        for t in range(q.shape[1] // DH):
            q_v[head0 + t, rows, :] = q[:, t * DH:(t + 1) * DH]

    for i in range(NX):
        rows = pl.ds(i * XC, XC)
        x_cps[i].wait()
        if i == 0:
            wq0_cp.wait()
        xf = x_v[rows, :].astype(F32)
        xc = xf - jnp.mean(xf, axis=1, keepdims=True)
        var = jnp.mean(xc * xc, axis=1, keepdims=True)
        hh = xc * lax.rsqrt(var + EPS) * (1.0 + mod_v[0:1, D:2 * D]) + mod_v[0:1, 0:D]
        hh = hh.astype(BF16)
        h_v[rows, :] = hh
        store_q(jnp.dot(hh, wq_v[:, 0:N0], preferred_element_type=F32), rows, 0)

    for c_ in kv_cps(0, 0):
        c_.start()
    for c_ in (wm2_cp, wr_cp, wo_cp, wg_cp, wu_cp, wd_cp):
        c_.start()

    wq1_cp.wait()

    def p1_body(j, carry):
        col0 = pl.multiple_of(N0 + j * 512, 512)
        w = wq_v[:, pl.ds(col0, 512)]
        for r in range(S // 512):
            rows = pl.ds(r * 512, 512)
            store_q(jnp.dot(h_v[rows, :], w, preferred_element_type=F32), rows, col0 // DH)
        return carry

    lax.fori_loop(0, (H * DH - N0) // 512, p1_body, 0)

    def p2_body(grp, carry):
        slot = grp % 2

        @pl.when(grp + 1 < H // G)
        def _():
            for c_ in kv_cps(grp + 1, 1 - slot):
                c_.start()

        for c_ in kv_cps(grp, slot):
            c_.wait()
        for hh in range(G):
            head = grp * G + hh
            for r in range(S // SUB):
                rows = pl.ds(r * SUB, SUB)
                o_v[head, rows, :] = _attn(q_v[head, rows, :], k_v[slot, hh], v_v[slot, hh])
        return carry

    lax.fori_loop(0, H // G, p2_body, 0)

    wm2_cp.wait()
    cols = pl.ds(2 * D, 4 * D)
    mod_v[:, cols] = jnp.dot(sc, wm_v[:, cols], preferred_element_type=F32)[:8]

    wo_cp.wait()
    wr_cp.wait()
    lane = lax.broadcasted_iota(jnp.int32, (8, 128), 1)

    def mod(i):
        return mod_v[0:1, i * D:(i + 1) * D]

    def out_cp(j, rows):
        return pltpu.make_async_copy(out_v.at[rows, :], out_hbm.at[rows, :], sems.at[_SEM["o0"] + j])

    def p3_body(j, carry):
        rows = pl.ds(pl.multiple_of(j * MC, MC), MC)
        acc = None
        for hh in range(H):
            d = jnp.dot(o_v[hh, rows, :], wo_v[hh * DH:(hh + 1) * DH, :], preferred_element_type=F32)
            acc = d if acc is None else acc + d
        x2 = x_v[rows, :].astype(F32) + mod(2) * acc
        x_v[rows, :] = x2.astype(BF16)
        xc = x2 - jnp.mean(x2, axis=1, keepdims=True)
        var = jnp.mean(xc * xc, axis=1, keepdims=True)
        cb1 = (1.0 + mod(4).astype(BF16).astype(F32)).astype(BF16).astype(F32)
        h2 = (xc * lax.rsqrt(var + EPS) * cb1 + mod(3)).astype(BF16)
        h_v[rows, :] = h2
        h2 = h2.astype(F32)
        out_v[rows, :] = (x2 + mod(5) * (h2 + h2 * 0.0)).astype(BF16)
        wr = wr_v[...].astype(F32)
        pr = None
        for t in range(D // 128):
            e = h2[:, t * 128:(t + 1) * 128] * wr[t:t + 1, :]
            pr = e if pr is None else pr + e
        r = jnp.sum(pr, axis=1, keepdims=True)
        rc = jnp.full((8, 128), -jnp.inf, F32)
        for i in range(MC // 8):
            rc = jnp.where(lane == i, r[8 * i:8 * i + 8, :], rc)
        r_v[j] = rc
        out_cp(j, rows).start()
        return carry

    lax.fori_loop(0, S // MC, p3_body, 0)

    nch = S // MC
    r = r_v[...].astype(BF16).astype(F32)
    tok = (lax.broadcasted_iota(jnp.int32, r.shape, 0) * MC + lax.broadcasted_iota(jnp.int32, r.shape, 2) * 8
           + lax.broadcasted_iota(jnp.int32, r.shape, 1))
    valid = lax.broadcasted_iota(jnp.int32, r.shape, 2) < MC // 8
    tokf = tok.astype(F32)

    def top1(cand):
        rr = jnp.where(cand, r, -jnp.inf)
        m = jnp.max(rr)
        i = jnp.min(jnp.where(cand & (rr == m), tokf, float(S)))
        return m, jnp.clip(i.astype(jnp.int32), 0, S - 1)

    m0, i0 = top1(valid)
    m1, i1 = top1(valid & (tok != i0))
    base = [pl.multiple_of((i // 16) * 16, 16) for i in (i0, i1)]
    xs = jnp.concatenate([h_v[pl.ds(b_, 16), :] for b_ in base], axis=0)

    wg_cp.wait()
    wu_cp.wait()
    g = jnp.dot(xs, wg_v[...], preferred_element_type=F32)
    u = jnp.dot(xs, wu_v[...], preferred_element_type=F32)
    act = (g * jax.nn.sigmoid(g) * u).astype(BF16)
    wd_cp.wait()
    y = jnp.dot(act, wd_v[...], preferred_element_type=F32)
    row16 = lax.broadcasted_iota(jnp.int32, (16, D), 0)
    g0 = jax.nn.sigmoid(jnp.full((16, D), m0, F32))
    g1 = jax.nn.sigmoid(jnp.full((16, D), m1, F32))
    for s_ in range(2):
        gate = jnp.where(row16 + base[s_] == i0, g0, jnp.where(row16 + base[s_] == i1, g1, 0.0))
        ys = y[16 * s_:16 * s_ + 16]
        upd = jnp.where((row16 + base[s_] == i0) | (row16 + base[s_] == i1), ys * gate, 0.0)
        h2 = xs[16 * s_:16 * s_ + 16].astype(F32)
        x2 = x_v[pl.ds(base[s_], 16), :].astype(F32)
        fix_v[s_] = (x2 + mod(5) * (h2 + (h2 * 0.0 + upd))).astype(BF16)

    for j in range(nch):
        out_cp(j, pl.ds(j * MC, MC)).wait()
    fix = [pltpu.make_async_copy(fix_v.at[s_], out_hbm.at[pl.ds(base[s_], 16), :], sems.at[_SEM["f0"] + s_])
           for s_ in range(2)]
    fix[0].start()

    @pl.when(base[0] != base[1])
    def _():
        fix[1].start()
        fix[1].wait()

    fix[0].wait()


@jax.jit
def pallas_adaLN_cond__mha_block_cached__moe_arch_mod__prompt_kernel(
    A_x: jax.Array,
    A_k_cache: jax.Array,
    A_v_cache: jax.Array,
    A_wq: jax.Array,
    A_wo: jax.Array,
    B_x: jax.Array,
    B_w_r: jax.Array,
    B_w_gate: jax.Array,
    B_w_up: jax.Array,
    B_w_down: jax.Array,
    c: jax.Array,
    w_mod: jax.Array,
):
    any_spec = pl.BlockSpec(memory_space=pl.ANY)
    vm = pltpu.VMEM
    out = pl.pallas_call(
        _kernel,
        name="adaln_mha_moe",
        in_specs=[any_spec] * 11,
        out_specs=any_spec,
        out_shape=jax.ShapeDtypeStruct((S, D), BF16),
        scratch_shapes=[
            vm((S, D), BF16),
            vm((S, D), BF16),
            vm((D, H * DH), BF16),
            vm((H, S, DH), BF16),
            vm((H, S, DH), BF16),
            vm((2, G, S, DH), BF16),
            vm((2, G, S, DH), BF16),
            vm((H * DH, D), BF16),
            vm((S, D), BF16),
            vm((8, 128), BF16),
            vm((D, FF), BF16),
            vm((D, FF), BF16),
            vm((FF, D), BF16),
            vm((1, D), BF16),
            vm((D, 6 * D), BF16),
            vm((8, 6 * D), F32),
            vm((S // MC, 8, 128), F32),
            vm((2, 16, D), BF16),
            pltpu.SemaphoreType.DMA((len(_names),)),
        ],
        compiler_params=pltpu.CompilerParams(vmem_limit_bytes=120 * 1024 * 1024),
    )(
        A_x.reshape(S, D), A_k_cache.reshape(H, S, DH), A_v_cache.reshape(H, S, DH), A_wq, A_wo,
        B_w_r.reshape(8, 128), B_w_gate, B_w_up, B_w_down, c, w_mod,
    )
    return out.reshape(1, S, D)
```

```python
import functools
import math

import jax
import jax.numpy as jnp
from jax import lax
from jax.experimental import pallas as pl
from jax.experimental.pallas import tpu as pltpu

F32 = jnp.float32
BF16 = jnp.bfloat16

S = 2048
D = 1024
H = 32
DH = 128
FF = 3584
EPS = 1e-5
QSCALE = (DH ** -0.5) * math.log2(math.e)

G = 2
SUB = 512
N0 = 512
N1 = 512
XC = 256
NX = S // XC
MC = 128
NM = S // MC
RG = MC // 8
PIECES = {1: [0], 2: [1], 3: [2], 4: [3], 5: [4], 6: [5], 7: [6, 7]}
FB = 512
NT = (((1,), (1,)), ((), ()))

_names = (["c", "wr", "wq0", "wq1", "wg", "wu", "wd", "wo", "wm2", "f0", "f1"]
          + ["wm%d" % i for i in range(4, 8)] + ["x%d" % i for i in range(NX)]
          + ["k0", "k1", "v0", "v1"] + ["o%d" % i for i in range(NM)])
_SEM = {n: i for i, n in enumerate(_names)}


def _attn(q, k, v):
    s = lax.dot_general(q, k, NT, preferred_element_type=F32)
    m = jnp.max(s, axis=1, keepdims=True)
    p = jnp.exp2(s - m)
    grp = 4
    acc = None
    tiles = []
    for g in range(S // (128 * grp)):
        ts = [p[:, (g * grp + j) * 128:(g * grp + j + 1) * 128] for j in range(grp)]
        t = (ts[0] + ts[1]) + (ts[2] + ts[3])
        acc = t if acc is None else acc + t
        tiles += ts[:-1] + [jnp.minimum(ts[-1], acc)]
    l = jnp.sum(acc, axis=1, keepdims=True)
    o = jnp.dot(jnp.concatenate(tiles, axis=1).astype(BF16), v, preferred_element_type=F32)
    return (o * pl.reciprocal(l, approx=True)).astype(BF16)


def _layernorm(x):
    xc = x - jnp.mean(x, axis=1, keepdims=True)
    var = jnp.mean(xc * xc, axis=1, keepdims=True)
    return xc * lax.rsqrt(var + EPS)


def _blk(i, n):
    return pl.ds(i * n if isinstance(i, int) else pl.multiple_of(i * n, n), n)


def _kernel(x_hbm, k_hbm, v_hbm, wq_hbm, wo_hbm, wr_hbm, wg_hbm, wu_hbm, wd_hbm,
            c_hbm, wm_hbm, out_hbm,
            x_v, h_v, p0, p1, p2, p3, p4, p5, p6, p7, wq_v, q_v, o_v, k_v, v_v, wo_v, wr_v, wg_v, wu_v, wd_v, c_v,
            wm_v, mod_v, acc_v, r_v, sel_v, fix_v, sems):

    piece = [p0, p1, p2, p3, p4, p5, p6, p7]

    def after_piece(t, p, r):
        z = piece[p][0:RG, 2 * D:2 * D + 128].astype(F32)
        z = lax.bitcast_convert_type(
            lax.bitcast_convert_type(z, jnp.int32) & lax.bitcast_convert_type(jnp.broadcast_to(r, z.shape), jnp.int32), F32)
        return (t.astype(F32) + jnp.tile(z, (t.shape[0] // RG, 1))).astype(BF16)

    def cp(name, src, dst, i=0):
        return pltpu.make_async_copy(src, dst, sems.at[_SEM[name] + i])

    def mod(i):
        return mod_v[0:1, i * D:(i + 1) * D]

    c_cp = cp("c", c_hbm, c_v)
    def wm_cp(i):
        return cp("wm4", wm_hbm.at[:, _blk(i, 512)], wm_v.at[:, _blk(i, 512)], i)
    wm2_cp = cp("wm2", wm_hbm.at[:, pl.ds(2 * D, 4 * D)], wm_v.at[:, pl.ds(2 * D, 4 * D)])
    def x_cp(i):
        return cp("x0", x_hbm.at[_blk(i, XC), :], x_v.at[_blk(i, XC), :], i)
    wq0_cp = cp("wq0", wq_hbm.at[:, pl.ds(0, N0)], wq_v.at[:, pl.ds(0, N0)])
    wq1_cp = cp("wq1", wq_hbm.at[:, pl.ds(N0, H * DH - N0)], wq_v.at[:, pl.ds(N0, H * DH - N0)])
    wo_cp = cp("wo", wo_hbm, wo_v)
    wr_cp = cp("wr", wr_hbm, wr_v)
    wg_cp = cp("wg", wg_hbm, wg_v)
    wu_cp = cp("wu", wu_hbm, wu_v)
    wd_cp = cp("wd", wd_hbm, wd_v)
    def out_cps(j):
        return [cp("o0", piece[p].at[_blk(j, RG), pl.ds(D, D)],
                   out_hbm.at[pl.ds(pl.multiple_of(j * MC + p * RG, RG), RG), :], j) for p in range(8)]

    def kv_cps(grp, slot):
        heads = pl.ds(grp * G, G)
        return (cp("k0", k_hbm.at[heads], k_v.at[slot], slot), cp("v0", v_hbm.at[heads], v_v.at[slot], slot))

    c_cp.start()
    for i in range(4):
        wm_cp(i).start()
    x_cp(0).start()
    wq0_cp.start()
    for i in range(1, NX):
        x_cp(i).start()
    wq1_cp.start()

    for p_ in piece:
        p_[0:RG, 2 * D:2 * D + 128] = jnp.zeros((RG, 128), BF16)
    c_cp.wait()
    cf = c_v[...].astype(F32)
    sc = jnp.broadcast_to(cf * jax.nn.sigmoid(cf), (16, D)).astype(BF16)

    def mod_body(i, carry):
        wm_cp(i).wait()
        mod_v[:, _blk(i, 512)] = jnp.dot(sc, wm_v[:, _blk(i, 512)], preferred_element_type=F32)[:8]
        return carry

    lax.fori_loop(0, 4, mod_body, 0)

    def store_q(q, rows, head0):
        q = (q * QSCALE).astype(BF16)
        for t in range(q.shape[1] // DH):
            q_v[head0 + t, rows, :] = q[:, t * DH:(t + 1) * DH]

    def ln1(i):
        rows = _blk(i, XC)
        h_v[rows, :] = (_layernorm(x_v[rows, :].astype(F32)) * (1.0 + mod(1)) + mod(0)).astype(BF16)

    x_cp(0).wait()
    ln1(0)
    wq0_cp.wait()

    def p1a_body(i, carry):
        @pl.when(i + 1 < NX)
        def _():
            x_cp(i + 1).wait()
        nxt = jnp.minimum(i + 1, NX - 1)
        for half in range(2):
            if half == 1:
                ln1(nxt)
            rows = pl.ds(pl.multiple_of(i * XC + half * (XC // 2), XC // 2), XC // 2)
            store_q(jnp.dot(h_v[rows, :], wq_v[:, 0:N0], preferred_element_type=F32), rows, 0)
        return carry

    lax.fori_loop(0, NX, p1a_body, 0)

    for c_ in kv_cps(0, 0):
        c_.start()
    for c_ in (wm2_cp, wr_cp, wo_cp, wg_cp, wu_cp, wd_cp):
        c_.start()

    wq1_cp.wait()

    def p1b_body(j, carry):
        w = wq_v[:, pl.ds(pl.multiple_of(N0 + j * N1, 128), N1)]
        for r in range(S // 512):
            rows = pl.ds(r * 512, 512)
            store_q(jnp.dot(h_v[rows, :], w, preferred_element_type=F32), rows, N0 // DH + j * (N1 // DH))
        return carry

    lax.fori_loop(0, (H * DH - N0) // N1, p1b_body, 0)

    def p2_body(grp, carry):
        slot = grp % 2

        @pl.when(grp + 1 < H // G)
        def _():
            for c_ in kv_cps(grp + 1, 1 - slot):
                c_.start()

        for c_ in kv_cps(grp, slot):
            c_.wait()
        for hh in range(G):
            head = grp * G + hh
            for r in range(S // SUB):
                rows = pl.ds(r * SUB, SUB)
                o_v[rows, _blk(head, DH)] = _attn(q_v[head, rows, :], k_v[slot, hh], v_v[slot, hh])
        return carry

    lax.fori_loop(0, H // G, p2_body, 0)

    wm2_cp.wait()

    def mod2_body(i, carry):
        mod_v[:, _blk(i, D)] = jnp.dot(sc, wm_v[:, _blk(i, D)], preferred_element_type=F32)[:8]
        return carry

    lax.fori_loop(2, 6, mod2_body, 0)
    mod_v[:, 4 * D:5 * D] = (1.0 + mod_v[:, 4 * D:5 * D].astype(BF16).astype(F32)).astype(BF16).astype(F32)

    wo_cp.wait()
    wr_cp.wait()
    lane = lax.broadcasted_iota(jnp.int32, (8, 128), 1)
    acc_v[0] = jnp.zeros((MC, D), F32)

    def finish(j, p, acc):
        rows = pl.ds(pl.multiple_of(j * MC + p * RG, RG), RG)
        x2 = x_v[rows, :].astype(F32) + mod(2) * acc[p * RG:(p + 1) * RG, :]
        h2 = (_layernorm(x2) * mod(4) + mod(3)).astype(BF16)
        piece[p][_blk(j, RG), 0:D] = h2
        h2 = h2.astype(F32)
        piece[p][_blk(j, RG), D:2 * D] = (x2 + mod(5) * (h2 + h2 * 0.0)).astype(BF16)
        wr = wr_v[...].astype(F32)
        pr = None
        for t in range(D // 128):
            e = h2[:, t * 128:(t + 1) * 128] * wr[t:t + 1, :]
            pr = e if pr is None else pr + e
        r = jnp.sum(pr, axis=1, keepdims=True)
        r_v[p] = jnp.where(lane == 2 * j, r[0:8], jnp.where(lane == 2 * j + 1, r[8:16], r_v[p]))
        return r

    def p3_body(j, carry):
        jp = jnp.maximum(j - 1, 0)
        rows = _blk(j, MC)
        accs = acc_v.at[pl.ds(j, 2)]
        for n in range(D // 128):
            cols = slice(n * 128, (n + 1) * 128)
            lhs = o_v[rows, :]
            tiles = [lhs[:, t * 128:(t + 1) * 128] for t in range(H)]
            for p in PIECES.get(n, ()):
                tiles[p] = after_piece(tiles[p], p, finish(jp, p, accs.at[0]))
            accs[1, :, cols] = jnp.dot(jnp.concatenate(tiles, axis=1), wo_v[:, cols], preferred_element_type=F32)

        @pl.when(j > 0)
        def _():
            for c_ in out_cps(j - 1):
                c_.start()
        return carry

    r_v[...] = jnp.zeros_like(r_v)
    lax.fori_loop(0, NM, p3_body, 0)
    for p in range(8):
        finish(NM - 1, p, acc_v.at[NM])
    for c_ in out_cps(NM - 1):
        c_.start()

    r = r_v[...].astype(BF16).astype(F32)
    ln_ = lax.broadcasted_iota(jnp.int32, r.shape, 2)
    tok = (lax.broadcasted_iota(jnp.int32, r.shape, 0) * RG + (ln_ // 2) * MC + (ln_ % 2) * 8
           + lax.broadcasted_iota(jnp.int32, r.shape, 1))
    valid = ln_ < 2 * NM
    tokf = tok.astype(F32)

    def top1(cand):
        rr = jnp.where(cand, r, -jnp.inf)
        m = jnp.max(rr)
        i = jnp.min(jnp.where(cand & (rr == m), tokf, float(S)))
        return m, jnp.clip(i.astype(jnp.int32), 0, S - 1)

    m0, i0 = top1(valid)
    m1, i1 = top1(valid & (tok != i0))
    base = [pl.multiple_of((i // RG) * RG, RG) for i in (i0, i1)]
    for s_, b_ in enumerate(base):
        for p in range(8):
            @pl.when((b_ % MC) // RG == p)
            def _(s_=s_, b_=b_, p=p):
                sel_v[s_] = piece[p][_blk(b_ // MC, RG), 0:2 * D]
    xs = jnp.concatenate([sel_v[0, :, 0:D], sel_v[1, :, 0:D]], axis=0)

    wg_cp.wait()
    wu_cp.wait()
    wd_cp.wait()

    def mlp_body(f, y):
        cols = _blk(f, FB)
        g = jnp.dot(xs, wg_v[:, cols], preferred_element_type=F32)
        u = jnp.dot(xs, wu_v[:, cols], preferred_element_type=F32)
        act = (g * jax.nn.sigmoid(g) * u).astype(BF16)
        return y + jnp.dot(act, wd_v[cols, :], preferred_element_type=F32)

    y = lax.fori_loop(0, FF // FB, mlp_body, jnp.zeros((32, D), F32))
    row16 = lax.broadcasted_iota(jnp.int32, (16, D), 0)
    g0 = jax.nn.sigmoid(jnp.full((16, D), m0, F32))
    g1 = jax.nn.sigmoid(jnp.full((16, D), m1, F32))
    for s_ in range(2):
        gate = jnp.where(row16 + base[s_] == i0, g0, jnp.where(row16 + base[s_] == i1, g1, 0.0))
        ys = y[16 * s_:16 * s_ + 16]
        upd = jnp.where((row16 + base[s_] == i0) | (row16 + base[s_] == i1), ys * gate, 0.0)
        fix_v[s_] = (sel_v[s_, :, D:2 * D].astype(F32) + mod(5) * upd).astype(BF16)

    def drain(j, carry):
        for c_ in out_cps(j):
            c_.wait()
        return carry

    lax.fori_loop(0, NM, drain, 0)
    fix = [cp("f0", fix_v.at[s_], out_hbm.at[pl.ds(base[s_], 16), :], s_) for s_ in range(2)]
    fix[0].start()

    @pl.when(base[0] != base[1])
    def _():
        fix[1].start()
        fix[1].wait()

    fix[0].wait()


@jax.jit
def pallas_adaLN_cond__mha_block_cached__moe_arch_mod__prompt_kernel(
    A_x: jax.Array,
    A_k_cache: jax.Array,
    A_v_cache: jax.Array,
    A_wq: jax.Array,
    A_wo: jax.Array,
    B_x: jax.Array,
    B_w_r: jax.Array,
    B_w_gate: jax.Array,
    B_w_up: jax.Array,
    B_w_down: jax.Array,
    c: jax.Array,
    w_mod: jax.Array,
):
    any_spec = pl.BlockSpec(memory_space=pl.ANY)
    vm = pltpu.VMEM
    out = pl.pallas_call(
        _kernel,
        name="adaln_mha_moe",
        in_specs=[any_spec] * 11,
        out_specs=any_spec,
        out_shape=jax.ShapeDtypeStruct((S, D), BF16),
        scratch_shapes=[
            vm((S, D), BF16),
            vm((S, D), BF16),
            *[vm((NM * RG, 2 * D + 128), BF16)] * 8,
            vm((D, H * DH), BF16),
            vm((H, S, DH), BF16),
            vm((S, H * DH), BF16),
            vm((2, G, S, DH), BF16),
            vm((2, G, S, DH), BF16),
            vm((H * DH, D), BF16),
            vm((8, 128), BF16),
            vm((D, FF), BF16),
            vm((D, FF), BF16),
            vm((FF, D), BF16),
            vm((1, D), BF16),
            vm((D, 6 * D), BF16),
            vm((8, 6 * D), F32),
            vm((NM + 1, MC, D), F32),
            vm((8, 8, 128), F32),
            vm((2, RG, 2 * D), BF16),
            vm((2, 16, D), BF16),
            pltpu.SemaphoreType.DMA((len(_names),)),
        ],
        compiler_params=pltpu.CompilerParams(vmem_limit_bytes=124 * 1024 * 1024),
    )(
        A_x.reshape(S, D), A_k_cache.reshape(H, S, DH), A_v_cache.reshape(H, S, DH), A_wq, A_wo,
        B_w_r.reshape(8, 128), B_w_gate, B_w_up, B_w_down, c, w_mod,
    )
    return out.reshape(1, S, D)
```

```python
import functools
import math

import jax
import jax.numpy as jnp
from jax import lax
from jax.experimental import pallas as pl
from jax.experimental.pallas import tpu as pltpu

F32 = jnp.float32
BF16 = jnp.bfloat16

S = 2048
D = 1024
H = 32
DH = 128
FF = 3584
EPS = 1e-5
QSCALE = (DH ** -0.5) * math.log2(math.e)

G = 2
SUBS = ((256, 384, 384, 512, 512), (512, 512, 384, 384, 256))
N0 = 512
N1 = 512
XC = 256
NX = S // XC
NH = 16
HG = XC // NH
MC = 128
NM = S // MC
RG = MC // 8
PIECES = {1: [0], 2: [1], 3: [2], 4: [3], 5: [4], 6: [5], 7: [6, 7]}
LN_PIECES = {3: [0], 4: [1], 5: [2], 6: [3], 7: [4], 8: [5], 9: [6], 10: [7], 11: [8], 12: [9], 13: [10, 11], 14: [12, 13], 15: [14, 15]}
FB = 512
NT = (((1,), (1,)), ((), ()))

_names = (["c", "wr", "wg", "wu", "wd", "wo", "wm2", "f0", "f1"]
          + ["wq%d" % i for i in range(8)] + ["wm%d" % i for i in range(4, 8)] + ["x%d" % i for i in range(NX)]
          + ["k0", "k1", "v0", "v1"] + ["o%d" % i for i in range(NM)])
_SEM = {n: i for i, n in enumerate(_names)}


def _attn(q, k, v):
    s = lax.dot_general(q, k, NT, preferred_element_type=F32)
    m = jnp.max(s, axis=1, keepdims=True)
    p = jnp.exp2(s - m)
    grp = 4
    acc = None
    tiles = []
    for g in range(S // (128 * grp)):
        ts = [p[:, (g * grp + j) * 128:(g * grp + j + 1) * 128] for j in range(grp)]
        t = (ts[0] + ts[1]) + (ts[2] + ts[3])
        acc = t if acc is None else acc + t
        tiles += ts[:-1] + [jnp.minimum(ts[-1], acc)]
    l = jnp.sum(acc, axis=1, keepdims=True)
    o = jnp.dot(jnp.concatenate(tiles, axis=1).astype(BF16), v, preferred_element_type=F32)
    return (o * pl.reciprocal(l, approx=True)).astype(BF16)


def _layernorm(x):
    xc = x - jnp.mean(x, axis=1, keepdims=True)
    var = jnp.mean(xc * xc, axis=1, keepdims=True)
    return xc * lax.rsqrt(var + EPS)


def _blk(i, n):
    return pl.ds(i * n if isinstance(i, int) else pl.multiple_of(i * n, n), n)


def _kernel(x_hbm, k_hbm, v_hbm, wq_hbm, wo_hbm, wr_hbm, wg_hbm, wu_hbm, wd_hbm,
            c_hbm, wm_hbm, out_hbm,
            x_v, wq_v, q_v, o_v, k_v, v_v, wo_v, wr_v, wg_v, wu_v, wd_v, c_v,
            wm_v, mod_v, acc_v, r_v, sel_v, fix_v, sems, *bufs):

    piece = bufs[NH:]

    def after(t, z, r=None):
        z = z.astype(F32)
        if r is not None:
            z = lax.bitcast_convert_type(
                lax.bitcast_convert_type(z, jnp.int32)
                & lax.bitcast_convert_type(jnp.broadcast_to(r, z.shape), jnp.int32), F32)
        return (t.astype(F32) + z).astype(BF16)

    def modt(i, t, rows):
        m = mod_v[:, i * D + t * 128:i * D + (t + 1) * 128]
        return jnp.concatenate([m] * (rows // 8), axis=0)

    hbuf = bufs[:NH]

    def cp(name, src, dst, i=0):
        return pltpu.make_async_copy(src, dst, sems.at[_SEM[name] + i])

    def mod(i):
        return mod_v[0:1, i * D:(i + 1) * D]

    c_cp = cp("c", c_hbm, c_v)
    def wm_cp(i):
        return cp("wm4", wm_hbm.at[:, _blk(i, 512)], wm_v.at[:, _blk(i, 512)], i)
    wm2_cp = cp("wm2", wm_hbm.at[:, pl.ds(2 * D, 4 * D)], wm_v.at[:, pl.ds(2 * D, 4 * D)])
    def x_cp(i):
        return cp("x0", x_hbm.at[_blk(i, XC), :], x_v.at[_blk(i, XC), :], i)
    def wq_cps(j):
        return [cp("wq0", wq_hbm.at[:, _blk(j * 4 + t, DH)], wq_v.at[j * 4 + t], j) for t in range(4)]
    wo_cps = [cp("wo", wo_hbm.at[:, pl.ds(n * 128, 128)], wo_v.at[n]) for n in range(D // 128)]
    wr_cp = cp("wr", wr_hbm, wr_v)
    wg_cp = cp("wg", wg_hbm, wg_v)
    wu_cp = cp("wu", wu_hbm, wu_v)
    wd_cp = cp("wd", wd_hbm, wd_v)
    out4 = out_hbm.reshape(NM, 8, RG, D)

    def out_cps(half):
        js = pl.ds(half * (NM // 2), NM // 2)
        return [cp("o0", piece[p].at[js, :, pl.ds(D, D)], out4.at[js, p], half * 8 + p) for p in range(8)]

    def kv_cps(grp, slot):
        heads = pl.ds(grp * G, G)
        return (cp("k0", k_hbm.at[heads], k_v.at[slot], slot), cp("v0", v_hbm.at[heads], v_v.at[slot], slot))

    c_cp.start()
    for i in range(4):
        wm_cp(i).start()
    x_cp(0).start()
    for c_ in wq_cps(0):
        c_.start()
    for i in range(1, NX):
        x_cp(i).start()
    for j_ in range(1, 8):
        for c_ in wq_cps(j_):
            c_.start()

    for p_ in hbuf:
        p_[D // 128, 0:16, :] = jnp.zeros((16, 128), BF16)
    for p_ in piece:
        p_[NM, :, 0:128] = jnp.zeros((RG, 128), BF16)
    c_cp.wait()
    cf = c_v[...].astype(F32)
    sc = jnp.broadcast_to(cf * jax.nn.sigmoid(cf), (16, D)).astype(BF16)

    def mod_body(i, carry):
        wm_cp(i).wait()
        mod_v[:, _blk(i, 512)] = jnp.dot(sc, wm_v[:, _blk(i, 512)], preferred_element_type=F32)[:8]
        return carry

    lax.fori_loop(0, 4, mod_body, 0)

    def ln1(i, p, dst, row0):
        rows = pl.ds(pl.multiple_of(i * XC + p * HG, HG), HG)
        xn = _layernorm(x_v[rows, :].astype(F32))
        for t in range(D // 128):
            dst[t, row0:row0 + HG, :] = (xn[:, t * 128:(t + 1) * 128] * modt(1, t, HG) + modt(0, t, HG)).astype(BF16)

    mod_v[:, D:2 * D] = 1.0 + mod_v[:, D:2 * D]
    x_cp(0).wait()
    for p in range(NH):
        ln1(0, p, hbuf[p], 0)
    for c_ in wq_cps(0):
        c_.wait()

    def p1a_body(i, carry):
        @pl.when(i + 1 < NX)
        def _():
            x_cp(i + 1).wait()
        nxt = jnp.minimum(i + 1, NX - 1)
        hv = [h.at[:, pl.ds(pl.multiple_of(i * HG, HG), 2 * HG), :] for h in hbuf]
        pos = 0
        for n in range(N0 // 128):
            for hf in range(2):
                wt = [wq_v[n, t * 128:(t + 1) * 128, :] for t in range(D // 128)]
                for half_ in range(2):
                    for c_, p in enumerate(LN_PIECES.get(pos, ())):
                        ln1(nxt, p, hv[p], HG)
                        t = 4 * half_ + c_
                        wt[t] = jnp.concatenate([after(wq_v[n, t * 128:t * 128 + 16, :], hbuf[p][D // 128, 0:16, :]),
                                                 wq_v[n, t * 128 + 16:(t + 1) * 128, :]], axis=0)
                    pos += 1
                lhs = jnp.concatenate(
                    [jnp.concatenate([hv[p][t, 0:HG, :] for t in range(D // 128)], axis=1)
                     for p in range(hf * NH // 2, (hf + 1) * NH // 2)], axis=0)
                q = jnp.dot(lhs, jnp.concatenate(wt, axis=0), preferred_element_type=F32)
                q_v[n, pl.ds(pl.multiple_of(i * XC + hf * (XC // 2), XC // 2), XC // 2), :] = (q * QSCALE).astype(BF16)
        return carry

    lax.fori_loop(0, NX, p1a_body, 0)

    for c_ in kv_cps(0, 0):
        c_.start()
    for c_ in (wm2_cp, wr_cp, *wo_cps, wg_cp, wu_cp, wd_cp):
        c_.start()

    def p1b_body(j, carry):
        for c_ in wq_cps(j):
            c_.wait()
        w = jnp.concatenate([wq_v[j * 4 + t] for t in range(4)], axis=1)
        for r in range(S // 512):
            lhs = jnp.concatenate(
                [jnp.concatenate([hbuf[p][t, i * HG:(i + 1) * HG, :] for t in range(D // 128)], axis=1)
                 for i in (2 * r, 2 * r + 1) for p in range(NH)], axis=0)
            q = jnp.dot(lhs, w, preferred_element_type=F32) * QSCALE
            for t in range(4):
                q_v[j * 4 + t, r * 512:(r + 1) * 512, :] = q[:, t * DH:(t + 1) * DH].astype(BF16)
        return carry

    lax.fori_loop(1, 8, p1b_body, 0)

    def p2_body(grp, carry):
        slot = grp % 2

        @pl.when(grp + 1 < H // G)
        def _():
            for c_ in kv_cps(grp + 1, 1 - slot):
                c_.start()

        for c_ in kv_cps(grp, slot):
            c_.wait()
        for hh in range(G):
            head = grp * G + hh
            r0 = 0
            for nr in SUBS[hh]:
                rows = pl.ds(r0, nr)
                r0 += nr
                o_v[head, rows, :] = _attn(q_v[head, rows, :], k_v[slot, hh], v_v[slot, hh])
        return carry

    lax.fori_loop(0, H // G, p2_body, 0)

    wm2_cp.wait()

    def mod2_body(i, carry):
        mod_v[:, _blk(i, D)] = jnp.dot(sc, wm_v[:, _blk(i, D)], preferred_element_type=F32)[:8]
        return carry

    lax.fori_loop(2, 6, mod2_body, 0)
    mod_v[:, 4 * D:5 * D] = (1.0 + mod_v[:, 4 * D:5 * D].astype(BF16).astype(F32)).astype(BF16).astype(F32)

    for c_ in wo_cps:
        c_.wait()
    wr_cp.wait()
    lane = lax.broadcasted_iota(jnp.int32, (8, 128), 1)
    acc_v[0] = jnp.zeros((MC, D), F32)

    def finish(j, p, acc):
        rows = pl.ds(pl.multiple_of(j * MC + p * RG, RG), RG)
        x2 = x_v[rows, :].astype(F32) + mod(2) * acc[p * RG:(p + 1) * RG, :]
        h2 = (_layernorm(x2) * mod(4) + mod(3)).astype(BF16)
        piece[p][j, :, 0:D] = h2
        h2 = h2.astype(F32)
        piece[p][j, :, D:2 * D] = (x2 + mod(5) * (h2 + h2 * 0.0)).astype(BF16)
        wr = wr_v[...].astype(F32)
        pr = None
        for t in range(D // 128):
            e = h2[:, t * 128:(t + 1) * 128] * wr[t:t + 1, :]
            pr = e if pr is None else pr + e
        r = jnp.sum(pr, axis=1, keepdims=True)
        r_v[p] = jnp.where(lane == 2 * j, r[0:8], jnp.where(lane == 2 * j + 1, r[8:16], r_v[p]))
        return r

    def p3_body(j, carry):
        jp = jnp.maximum(j - 1, 0)
        accs = acc_v.at[pl.ds(j, 2)]
        for n in range(D // 128):
            cols = slice(n * 128, (n + 1) * 128)
            row0 = pl.multiple_of(j * MC, MC)
            tiles = [o_v[h, pl.ds(row0, MC), :] for h in range(H)]
            for p in PIECES.get(n, ()):
                r = finish(jp, p, accs.at[0])
                tiles[p] = jnp.concatenate([after(o_v[p, pl.ds(row0, 16), :], piece[p][NM, :, 0:128], r),
                                            o_v[p, pl.ds(row0 + 16, MC - 16), :]], axis=0)
            lhs = jnp.concatenate(tiles, axis=1)
            accs[1, :, cols] = jnp.dot(lhs, wo_v[n], preferred_element_type=F32)

        @pl.when(j == NM // 2)
        def _():
            for c_ in out_cps(0):
                c_.start()
        return carry

    r_v[...] = jnp.zeros_like(r_v)
    lax.fori_loop(0, NM, p3_body, 0)
    for p in range(8):
        finish(NM - 1, p, acc_v.at[NM])
    for c_ in out_cps(1):
        c_.start()

    r = r_v[...].astype(BF16).astype(F32)
    ln_ = lax.broadcasted_iota(jnp.int32, r.shape, 2)
    tok = (lax.broadcasted_iota(jnp.int32, r.shape, 0) * RG + (ln_ // 2) * MC + (ln_ % 2) * 8
           + lax.broadcasted_iota(jnp.int32, r.shape, 1))
    valid = ln_ < 2 * NM
    tokf = tok.astype(F32)

    def top1(cand):
        rr = jnp.where(cand, r, -jnp.inf)
        m = jnp.max(rr)
        i = jnp.min(jnp.where(cand & (rr == m), tokf, float(S)))
        return m, jnp.clip(i.astype(jnp.int32), 0, S - 1)

    m0, i0 = top1(valid)
    m1, i1 = top1(valid & (tok != i0))
    base = [pl.multiple_of((i // RG) * RG, RG) for i in (i0, i1)]
    for s_, b_ in enumerate(base):
        for p in range(8):
            @pl.when((b_ % MC) // RG == p)
            def _(s_=s_, b_=b_, p=p):
                sel_v[s_] = piece[p][b_ // MC]
    xs = jnp.concatenate([sel_v[0, :, 0:D], sel_v[1, :, 0:D]], axis=0)

    wg_cp.wait()
    wu_cp.wait()
    wd_cp.wait()

    def mlp_body(f, y):
        cols = _blk(f, FB)
        g = jnp.dot(xs, wg_v[:, cols], preferred_element_type=F32)
        u = jnp.dot(xs, wu_v[:, cols], preferred_element_type=F32)
        act = (g * jax.nn.sigmoid(g) * u).astype(BF16)
        return y + jnp.dot(act, wd_v[cols, :], preferred_element_type=F32)

    y = lax.fori_loop(0, FF // FB, mlp_body, jnp.zeros((32, D), F32))
    row16 = lax.broadcasted_iota(jnp.int32, (16, D), 0)
    g0 = jax.nn.sigmoid(jnp.full((16, D), m0, F32))
    g1 = jax.nn.sigmoid(jnp.full((16, D), m1, F32))
    for s_ in range(2):
        gate = jnp.where(row16 + base[s_] == i0, g0, jnp.where(row16 + base[s_] == i1, g1, 0.0))
        ys = y[16 * s_:16 * s_ + 16]
        upd = jnp.where((row16 + base[s_] == i0) | (row16 + base[s_] == i1), ys * gate, 0.0)
        fix_v[s_] = (sel_v[s_, :, D:2 * D].astype(F32) + mod(5) * upd).astype(BF16)

    for c_ in out_cps(0) + out_cps(1):
        c_.wait()
    fix = [cp("f0", fix_v.at[s_], out_hbm.at[pl.ds(base[s_], 16), :], s_) for s_ in range(2)]
    fix[0].start()

    @pl.when(base[0] != base[1])
    def _():
        fix[1].start()
        fix[1].wait()

    fix[0].wait()


@jax.jit
def pallas_adaLN_cond__mha_block_cached__moe_arch_mod__prompt_kernel(
    A_x: jax.Array,
    A_k_cache: jax.Array,
    A_v_cache: jax.Array,
    A_wq: jax.Array,
    A_wo: jax.Array,
    B_x: jax.Array,
    B_w_r: jax.Array,
    B_w_gate: jax.Array,
    B_w_up: jax.Array,
    B_w_down: jax.Array,
    c: jax.Array,
    w_mod: jax.Array,
):
    any_spec = pl.BlockSpec(memory_space=pl.ANY)
    vm = pltpu.VMEM
    out = pl.pallas_call(
        _kernel,
        name="adaln_mha_moe",
        in_specs=[any_spec] * 11,
        out_specs=any_spec,
        out_shape=jax.ShapeDtypeStruct((S, D), BF16),
        scratch_shapes=[
            vm((S, D), BF16),
            vm((H, D, DH), BF16),
            vm((H, S, DH), BF16),
            vm((H, S, DH), BF16),
            vm((2, G, S, DH), BF16),
            vm((2, G, S, DH), BF16),
            vm((D // 128, H * DH, 128), BF16),
            vm((8, 128), BF16),
            vm((D, FF), BF16),
            vm((D, FF), BF16),
            vm((FF, D), BF16),
            vm((1, D), BF16),
            vm((D, 6 * D), BF16),
            vm((8, 6 * D), F32),
            vm((NM + 1, MC, D), F32),
            vm((8, 8, 128), F32),
            vm((2, RG, 2 * D), BF16),
            vm((2, 16, D), BF16),
            pltpu.SemaphoreType.DMA((len(_names),)),
            *[vm((D // 128 + 1, (NX + 1) * HG, 128), BF16)] * NH,
            *[vm((NM + 1, RG, 2 * D), BF16)] * 8,
        ],
        compiler_params=pltpu.CompilerParams(vmem_limit_bytes=124 * 1024 * 1024),
    )(
        A_x.reshape(S, D), A_k_cache.reshape(H, S, DH), A_v_cache.reshape(H, S, DH), A_wq, A_wo,
        B_w_r.reshape(8, 128), B_w_gate, B_w_up, B_w_down, c, w_mod,
    )
    return out.reshape(1, S, D)
```

```python
import functools
import math

import jax
import jax.numpy as jnp
from jax import lax
from jax.experimental import pallas as pl
from jax.experimental.pallas import tpu as pltpu

F32 = jnp.float32
BF16 = jnp.bfloat16

S = 2048
D = 1024
H = 32
DH = 128
FF = 3584
EPS = 1e-5
QSCALE = (DH ** -0.5) * math.log2(math.e)

G = 2
SUBS = ((256, 384, 384, 512, 512), (512, 512, 384, 384, 256))
N0 = 512
N1 = 512
XC = 256
NX = S // XC
NH = 16
HG = XC // NH
MC = 128
NM = S // MC
RG = MC // 8
PIECES = {1: [0], 2: [1], 3: [2], 4: [3], 5: [4], 6: [5], 7: [6, 7]}
LN_PIECES = {3: [0], 4: [1], 5: [2], 6: [3], 7: [4], 8: [5], 9: [6], 10: [7], 11: [8], 12: [9], 13: [10, 11], 14: [12, 13], 15: [14, 15]}
MOD_PIECES = {0: [(0, 4)], 1: [(1, 0), (2, 4)], 2: [(3, 0), (4, 4)]}
MT = 5
FB = 512
NT = (((1,), (1,)), ((), ()))

_names = (["c", "wr", "wg", "wu", "wd", "wo", "f0", "f1"]
          + ["wq%d" % i for i in range(8)] + ["wn%d" % i for i in range(8)] + ["wm%d" % i for i in range(4, 8)] + ["x%d" % i for i in range(NX + 1)]
          + ["k0", "k1", "v0", "v1"] + ["o%d" % i for i in range(NM)])
_SEM = {n: i for i, n in enumerate(_names)}


def _attn(q, k, v):
    s = lax.dot_general(q, k, NT, preferred_element_type=F32)
    m = jnp.max(s, axis=1, keepdims=True)
    p = jnp.exp2(s - m)
    grp = 4
    acc = None
    tiles = []
    for g in range(S // (128 * grp)):
        ts = [p[:, (g * grp + j) * 128:(g * grp + j + 1) * 128] for j in range(grp)]
        t = (ts[0] + ts[1]) + (ts[2] + ts[3])
        acc = t if acc is None else acc + t
        tiles += ts[:-1] + [jnp.minimum(ts[-1], acc)]
    l = jnp.sum(acc, axis=1, keepdims=True)
    o = jnp.dot(jnp.concatenate(tiles, axis=1).astype(BF16), v, preferred_element_type=F32)
    return (o * pl.reciprocal(l, approx=True)).astype(BF16)


def _layernorm(x):
    xc = x - jnp.mean(x, axis=1, keepdims=True)
    var = jnp.mean(xc * xc, axis=1, keepdims=True)
    return xc * lax.rsqrt(var + EPS)


def _blk(i, n):
    return pl.ds(i * n if isinstance(i, int) else pl.multiple_of(i * n, n), n)


def _kernel(x_hbm, k_hbm, v_hbm, wq_hbm, wo_hbm, wr_hbm, wg_hbm, wu_hbm, wd_hbm,
            c_hbm, wm_hbm, out_hbm,
            x_v, wq_v, q_v, o_v, k_v, v_v, wo_v, wr_v, wg_v, wu_v, wd_v, c_v,
            wm_v, mod_v, scb_v, acc_v, r_v, sel_v, fix_v, sems, *bufs):

    piece = bufs[NH:NH + 8]
    mp = bufs[NH + 8:]

    def after(t, z, r=None):
        z = z.astype(F32)
        if r is not None:
            z = lax.bitcast_convert_type(
                lax.bitcast_convert_type(z, jnp.int32)
                & lax.bitcast_convert_type(jnp.broadcast_to(r, z.shape), jnp.int32), F32)
        return (t.astype(F32) + z).astype(BF16)

    def modt(i, t, rows):
        m = mod_v[:, i * D + t * 128:i * D + (t + 1) * 128]
        return jnp.concatenate([m] * (rows // 8), axis=0)

    hbuf = bufs[:NH]

    def cp(name, src, dst, i=0):
        return pltpu.make_async_copy(src, dst, sems.at[_SEM[name] + i])

    def modw(i, rows):
        return jnp.concatenate([mod_v[:, i * D:(i + 1) * D]] * (rows // 8), axis=0)

    def mod(i):
        return mod_v[0:1, i * D:(i + 1) * D]

    c_cp = cp("c", c_hbm, c_v)
    def wm_cp(i):
        return cp("wm4", wm_hbm.at[:, _blk(i, 512)], wm_v.at[:, _blk(i, 512)], i)
    def wm2_cp(j):
        return cp("wn0", wm_hbm.at[:, _blk(4 + j, 512)], wm_v.at[:, _blk(4 + j, 512)], j)
    def x_cp(i):
        return cp("x0", x_hbm.at[_blk(min(i, NX - 1) if isinstance(i, int) else jnp.minimum(i, NX - 1), XC), :],
                  x_v.at[_blk(i, XC), :], i)
    def wq_cps(j):
        return [cp("wq0", wq_hbm.at[:, _blk(j * 4 + t, DH)], wq_v.at[j * 4 + t], j) for t in range(4)]
    wo_cps = [cp("wo", wo_hbm.at[:, pl.ds(n * 128, 128)], wo_v.at[n]) for n in range(D // 128)]
    wr_cp = cp("wr", wr_hbm, wr_v)
    wg_cp = cp("wg", wg_hbm, wg_v)
    wu_cp = cp("wu", wu_hbm, wu_v)
    wd_cp = cp("wd", wd_hbm, wd_v)
    out4 = out_hbm.reshape(NM, 8, RG, D)

    def out_cps(half):
        js = pl.ds(0, NM // 2 - 1) if half == 0 else pl.ds(NM // 2 - 1, NM // 2 + 1)
        return [cp("o0", piece[p].at[js, :, pl.ds(D, D)], out4.at[js, p], half * 8 + p) for p in range(8)]

    def kv_cps(grp, slot):
        heads = pl.ds(grp * G, G)
        return (cp("k0", k_hbm.at[heads], k_v.at[slot], slot), cp("v0", v_hbm.at[heads], v_v.at[slot], slot))

    c_cp.start()
    for i in range(4):
        wm_cp(i).start()
    x_cp(0).start()
    for c_ in wq_cps(0):
        c_.start()
    x_cp(1).start()

    for p_ in hbuf:
        p_[D // 128, 0:16, :] = jnp.zeros((16, 128), BF16)
    for p_ in piece:
        p_[NM, :, 0:128] = jnp.zeros((RG, 128), BF16)
    c_cp.wait()
    cf = c_v[...].astype(F32)
    sc = jnp.broadcast_to(cf * jax.nn.sigmoid(cf), (16, D)).astype(BF16)
    scb_v[...] = jnp.broadcast_to(sc[0:1].astype(F32), (128, D)).T
    for m_ in mp:
        m_[7] = jnp.zeros((8, 128), F32)

    def mod_body(i, carry):
        wm_cp(i).wait()
        mod_v[:, _blk(i, 512)] = jnp.dot(sc, wm_v[:, _blk(i, 512)], preferred_element_type=F32)[:8]
        return carry

    lax.fori_loop(0, 4, mod_body, 0)

    def ln1(i, p, dst, row0):
        rows = pl.ds(pl.multiple_of(i * XC + p * HG, HG), HG)
        xn = _layernorm(x_v[rows, :].astype(F32))
        for t in range(D // 128):
            dst[t, row0:row0 + HG, :] = (xn[:, t * 128:(t + 1) * 128] * modt(1, t, HG) + modt(0, t, HG)).astype(BF16)

    mod_v[:, D:2 * D] = 1.0 + mod_v[:, D:2 * D]
    x_cp(0).wait()
    for p in range(NH):
        ln1(0, p, hbuf[p], 0)
    for c_ in wq_cps(0):
        c_.wait()
    for i in range(2, NX + 1):
        x_cp(i).start()
    wm2_cp(0).start()
    for j_ in range(1, 8):
        for c_ in wq_cps(j_):
            c_.start()
        wm2_cp(j_).start()

    def p1a_body(i, carry):
        nxt = i + 1
        x_cp(nxt).wait()
        hv = [h.at[:, pl.ds(pl.multiple_of(i * HG, HG), 2 * HG), :] for h in hbuf]
        pos = 0
        for n in range(N0 // 128):
            for hf in range(2):
                wt = [wq_v[n, t * 128:(t + 1) * 128, :] for t in range(D // 128)]
                for half_ in range(2):
                    for c_, p in enumerate(LN_PIECES.get(pos, ())):
                        ln1(nxt, p, hv[p], HG)
                        t = 4 * half_ + c_
                        wt[t] = jnp.concatenate([after(wq_v[n, t * 128:t * 128 + 16, :], hbuf[p][D // 128, 0:16, :]),
                                                 wq_v[n, t * 128 + 16:(t + 1) * 128, :]], axis=0)
                    pos += 1
                lhs = jnp.concatenate(
                    [jnp.concatenate([hv[p][t, 0:HG, :] for t in range(D // 128)], axis=1)
                     for p in range(hf * NH // 2, (hf + 1) * NH // 2)], axis=0)
                q = jnp.dot(lhs, jnp.concatenate(wt, axis=0), preferred_element_type=F32)
                q_v[n, pl.ds(pl.multiple_of(i * XC + hf * (XC // 2), XC // 2), XC // 2), :] = (q * QSCALE).astype(BF16)
        return carry

    lax.fori_loop(0, NX, p1a_body, 0)

    for c_ in kv_cps(0, 0):
        c_.start()
    for c_ in (wr_cp, *wo_cps, wg_cp, wu_cp, wd_cp):
        c_.start()

    wm2_cp(0).wait()

    def p1b_body(j, carry):
        for c_ in wq_cps(j):
            c_.wait()
        wm2_cp(j).wait()
        tile0 = jnp.minimum(MT * (j - 1), 32 - MT)
        for r in range(S // 512):
            wt = [[wq_v[j * 4 + t, k * 128:(k + 1) * 128, :] for k in range(D // 128)] for t in range(4)]
            for p, k in MOD_PIECES.get(r, ()):
                wm = wm_v[:, pl.ds(pl.multiple_of(2 * D + (tile0 + p) * 128, 128), 128)].astype(F32)
                mp[p][j - 1] = jnp.broadcast_to(jnp.sum(wm * scb_v[...], axis=0, keepdims=True), (8, 128))
                z = jnp.concatenate([mp[p][7]] * 2, axis=0)
                wt[0][k] = jnp.concatenate([after(wq_v[j * 4, k * 128:k * 128 + 16, :], z),
                                            wq_v[j * 4, k * 128 + 16:(k + 1) * 128, :]], axis=0)
            w = jnp.concatenate([jnp.concatenate(c_, axis=0) for c_ in wt], axis=1)
            lhs = jnp.concatenate(
                [jnp.concatenate([hbuf[p][t, i * HG:(i + 1) * HG, :] for t in range(D // 128)], axis=1)
                 for i in (2 * r, 2 * r + 1) for p in range(NH)], axis=0)
            q = jnp.dot(lhs, w, preferred_element_type=F32) * QSCALE
            for t in range(4):
                q_v[j * 4 + t, r * 512:(r + 1) * 512, :] = q[:, t * DH:(t + 1) * DH].astype(BF16)
        return carry

    lax.fori_loop(1, 8, p1b_body, 0)
    for c_ in range(32):
        j_ = min(c_ // MT, 6)
        mod_v[:, 2 * D + c_ * 128:2 * D + (c_ + 1) * 128] = mp[c_ - min(MT * j_, 32 - MT)][j_]

    def p2_body(grp, carry):
        slot = grp % 2

        for c_ in kv_cps(jnp.minimum(grp + 1, H // G - 1), 1 - slot):
            c_.start()
        for c_ in kv_cps(grp, slot):
            c_.wait()
        for hh in range(G):
            head = grp * G + hh
            r0 = 0
            for nr in SUBS[hh]:
                rows = pl.ds(r0, nr)
                r0 += nr
                o_v[head, rows, :] = _attn(q_v[head, rows, :], k_v[slot, hh], v_v[slot, hh])
        return carry

    lax.fori_loop(0, H // G, p2_body, 0)
    for c_ in kv_cps(H // G - 1, (H // G) % 2):
        c_.wait()

    mod_v[:, 4 * D:5 * D] = (1.0 + mod_v[:, 4 * D:5 * D].astype(BF16).astype(F32)).astype(BF16).astype(F32)

    for c_ in wo_cps:
        c_.wait()
    wr_cp.wait()
    wr = wr_v[...].astype(F32)
    for t in range(D // 128):
        mod_v[:, t * 128:(t + 1) * 128] = jnp.broadcast_to(wr[t:t + 1, :], (8, 128))
    lane = lax.broadcasted_iota(jnp.int32, (8, 128), 1)
    acc_v[0] = jnp.zeros((MC, D), F32)

    def finish(j, p, acc):
        rows = pl.ds(pl.multiple_of(j * MC + p * RG, RG), RG)
        x2 = x_v[rows, :].astype(F32) + modw(2, RG) * acc[p * RG:(p + 1) * RG, :]
        h2 = (_layernorm(x2) * modw(4, RG) + modw(3, RG)).astype(BF16)
        piece[p][j, :, 0:D] = h2
        h2 = h2.astype(F32)
        piece[p][j, :, D:2 * D] = (x2 + modw(5, RG) * (h2 + h2 * 0.0)).astype(BF16)
        e = h2 * modw(0, RG)
        pr = None
        for t in range(D // 128):
            pr = e[:, t * 128:(t + 1) * 128] if pr is None else pr + e[:, t * 128:(t + 1) * 128]
        r = jnp.sum(pr, axis=1, keepdims=True)
        r_v[p] = jnp.where(lane == 2 * j, r[0:8], jnp.where(lane == 2 * j + 1, r[8:16], r_v[p]))
        return r

    def p3_body(j, carry):
        jp = jnp.maximum(j - 1, 0)
        accs = acc_v.at[pl.ds(j, 2)]
        for n in range(D // 128):
            cols = slice(n * 128, (n + 1) * 128)
            row0 = pl.multiple_of(j * MC, MC)
            tiles = [o_v[h, pl.ds(row0, MC), :] for h in range(H)]
            for p in PIECES.get(n, ()):
                r = finish(jp, p, accs.at[0])
                tiles[p] = jnp.concatenate([after(o_v[p, pl.ds(row0, 16), :], piece[p][NM, :, 0:128], r),
                                            o_v[p, pl.ds(row0 + 16, MC - 16), :]], axis=0)
            lhs = jnp.concatenate(tiles, axis=1)
            accs[1, :, cols] = jnp.dot(lhs, wo_v[n], preferred_element_type=F32)

        return carry

    def p3_half(half, carry):
        lax.fori_loop(half * (NM // 2), (half + 1) * (NM // 2), p3_body, 0)

        @pl.when(half == 0)
        def _():
            for c_ in out_cps(0):
                c_.start()
        return carry

    r_v[...] = jnp.zeros_like(r_v)
    lax.fori_loop(0, 2, p3_half, 0)
    for p in range(8):
        finish(NM - 1, p, acc_v.at[NM])
    for c_ in out_cps(1):
        c_.start()

    r = r_v[...].astype(BF16).astype(F32)
    ln_ = lax.broadcasted_iota(jnp.int32, r.shape, 2)
    tok = (lax.broadcasted_iota(jnp.int32, r.shape, 0) * RG + (ln_ // 2) * MC + (ln_ % 2) * 8
           + lax.broadcasted_iota(jnp.int32, r.shape, 1))
    valid = ln_ < 2 * NM
    tokf = tok.astype(F32)

    def top1(cand):
        rr = jnp.where(cand, r, -jnp.inf)
        m = jnp.max(rr)
        i = jnp.min(jnp.where(cand & (rr == m), tokf, float(S)))
        return m, jnp.clip(i.astype(jnp.int32), 0, S - 1)

    m0, i0 = top1(valid)
    m1, i1 = top1(valid & (tok != i0))
    base = [pl.multiple_of((i // RG) * RG, RG) for i in (i0, i1)]
    for s_, b_ in enumerate(base):
        for p in range(8):
            @pl.when((b_ % MC) // RG == p)
            def _(s_=s_, b_=b_, p=p):
                sel_v[s_] = piece[p][b_ // MC]
    xs = jnp.concatenate([sel_v[0, :, 0:D], sel_v[1, :, 0:D]], axis=0)

    wg_cp.wait()
    wu_cp.wait()
    wd_cp.wait()

    def mlp_body(f, y):
        cols = _blk(f, FB)
        g = jnp.dot(xs, wg_v[:, cols], preferred_element_type=F32)
        u = jnp.dot(xs, wu_v[:, cols], preferred_element_type=F32)
        act = (g * jax.nn.sigmoid(g) * u).astype(BF16)
        return y + jnp.dot(act, wd_v[cols, :], preferred_element_type=F32)

    y = lax.fori_loop(0, FF // FB, mlp_body, jnp.zeros((32, D), F32))
    row16 = lax.broadcasted_iota(jnp.int32, (16, D), 0)
    g0 = jax.nn.sigmoid(jnp.full((16, D), m0, F32))
    g1 = jax.nn.sigmoid(jnp.full((16, D), m1, F32))
    for s_ in range(2):
        gate = jnp.where(row16 + base[s_] == i0, g0, jnp.where(row16 + base[s_] == i1, g1, 0.0))
        ys = y[16 * s_:16 * s_ + 16]
        upd = jnp.where((row16 + base[s_] == i0) | (row16 + base[s_] == i1), ys * gate, 0.0)
        fix_v[s_] = (sel_v[s_, :, D:2 * D].astype(F32) + mod(5) * upd).astype(BF16)

    for c_ in out_cps(0) + out_cps(1):
        c_.wait()
    fix = [cp("f0", fix_v.at[s_], out_hbm.at[pl.ds(base[s_], 16), :], s_) for s_ in range(2)]
    fix[0].start()

    @pl.when(base[0] != base[1])
    def _():
        fix[1].start()
        fix[1].wait()

    fix[0].wait()


@jax.jit
def pallas_adaLN_cond__mha_block_cached__moe_arch_mod__prompt_kernel(
    A_x: jax.Array,
    A_k_cache: jax.Array,
    A_v_cache: jax.Array,
    A_wq: jax.Array,
    A_wo: jax.Array,
    B_x: jax.Array,
    B_w_r: jax.Array,
    B_w_gate: jax.Array,
    B_w_up: jax.Array,
    B_w_down: jax.Array,
    c: jax.Array,
    w_mod: jax.Array,
):
    any_spec = pl.BlockSpec(memory_space=pl.ANY)
    vm = pltpu.VMEM
    out = pl.pallas_call(
        _kernel,
        name="adaln_mha_moe",
        in_specs=[any_spec] * 11,
        out_specs=any_spec,
        out_shape=jax.ShapeDtypeStruct((S, D), BF16),
        scratch_shapes=[
            vm((S + XC, D), BF16),
            vm((H, D, DH), BF16),
            vm((H, S, DH), BF16),
            vm((H, S, DH), BF16),
            vm((2, G, S, DH), BF16),
            vm((2, G, S, DH), BF16),
            vm((D // 128, H * DH, 128), BF16),
            vm((8, 128), BF16),
            vm((D, FF), BF16),
            vm((D, FF), BF16),
            vm((FF, D), BF16),
            vm((1, D), BF16),
            vm((D, 6 * D), BF16),
            vm((8, 6 * D), F32),
            vm((D, 128), F32),
            vm((NM + 1, MC, D), F32),
            vm((8, 8, 128), F32),
            vm((2, RG, 2 * D), BF16),
            vm((2, 16, D), BF16),
            pltpu.SemaphoreType.DMA((len(_names),)),
            *[vm((D // 128 + 1, (NX + 1) * HG, 128), BF16)] * NH,
            *[vm((NM + 1, RG, 2 * D), BF16)] * 8,
            *[vm((8, 8, 128), F32)] * MT,
        ],
        compiler_params=pltpu.CompilerParams(vmem_limit_bytes=124 * 1024 * 1024),
    )(
        A_x.reshape(S, D), A_k_cache.reshape(H, S, DH), A_v_cache.reshape(H, S, DH), A_wq, A_wo,
        B_w_r.reshape(8, 128), B_w_gate, B_w_up, B_w_down, c, w_mod,
    )
    return out.reshape(1, S, D)
```

```python
import functools
import math

import jax
import jax.numpy as jnp
from jax import lax
from jax.experimental import pallas as pl
from jax.experimental.pallas import tpu as pltpu

F32 = jnp.float32
BF16 = jnp.bfloat16

S = 2048
D = 1024
H = 32
DH = 128
FF = 3584
EPS = 1e-5
QSCALE = (DH ** -0.5) * math.log2(math.e)

G = 2
SUBS = ((256, 384, 384, 512, 512), (512, 512, 384, 384, 256))
N0 = 512
N1 = 512
XC = 256
NX = S // XC
NH = 16
HG = XC // NH
MC = 128
NM = S // MC
RG = MC // 8
PIECES = {1: [0], 2: [1], 3: [2], 4: [3], 5: [4], 6: [5], 7: [6, 7]}
LN_PIECES = {3: [0], 4: [1], 5: [2], 6: [3], 7: [4], 8: [5], 9: [6], 10: [7], 11: [8], 12: [9], 13: [10, 11], 14: [12, 13], 15: [14, 15]}
MOD_PIECES = {0: [(0, 4)], 1: [(1, 0), (2, 4)], 2: [(3, 0), (4, 4)]}
MT = 5
FB = 512
NT = (((1,), (1,)), ((), ()))

_names = (["c", "wr", "wg", "wu", "wd", "wo", "f0", "f1"]
          + ["wq%d" % i for i in range(8)] + ["wn%d" % i for i in range(8)] + ["wm%d" % i for i in range(4, 8)] + ["x%d" % i for i in range(NX + 1)]
          + ["k0", "k1", "v0", "v1"] + ["o%d" % i for i in range(NM)])
_SEM = {n: i for i, n in enumerate(_names)}


def _attn(q, k, v):
    s = lax.dot_general(q, k, NT, preferred_element_type=F32)
    m = jnp.max(s, axis=1, keepdims=True)
    p = jnp.exp2(s - m)
    grp = 4
    acc = None
    tiles = []
    for g in range(S // (128 * grp)):
        ts = [p[:, (g * grp + j) * 128:(g * grp + j + 1) * 128] for j in range(grp)]
        t = (ts[0] + ts[1]) + (ts[2] + ts[3])
        acc = t if acc is None else acc + t
        tiles += ts[:-1] + [jnp.minimum(ts[-1], acc)]
    l = jnp.sum(acc, axis=1, keepdims=True)
    o = jnp.dot(jnp.concatenate(tiles, axis=1).astype(BF16), v, preferred_element_type=F32)
    return (o * pl.reciprocal(l, approx=True)).astype(BF16)


def _layernorm(x):
    xc = x - jnp.mean(x, axis=1, keepdims=True)
    var = jnp.mean(xc * xc, axis=1, keepdims=True)
    return xc * lax.rsqrt(var + EPS)


def _blk(i, n):
    return pl.ds(i * n if isinstance(i, int) else pl.multiple_of(i * n, n), n)


def _kernel(x_hbm, k_hbm, v_hbm, wq_hbm, wo_hbm, wr_hbm, wg_hbm, wu_hbm, wd_hbm,
            c_hbm, wm_hbm, out_hbm,
            x_v, wq_v, q_v, o_v, k_v, v_v, wo_v, wr_v, wg_v, wu_v, wd_v, c_v,
            wm_v, mod_v, scb_v, acc_v, r_v, sel_v, fix_v, sems, *bufs):

    piece = bufs[NH:NH + 8]
    mp = bufs[NH + 8:]

    def after(t, z, r=None):
        z = z.astype(F32)
        if r is not None:
            z = lax.bitcast_convert_type(
                lax.bitcast_convert_type(z, jnp.int32)
                & lax.bitcast_convert_type(jnp.broadcast_to(r, z.shape), jnp.int32), F32)
        return (t.astype(F32) + z).astype(BF16)

    def modt(i, t, rows):
        m = mod_v[:, i * D + t * 128:i * D + (t + 1) * 128]
        return jnp.concatenate([m] * (rows // 8), axis=0)

    hbuf = bufs[:NH]

    def cp(name, src, dst, i=0):
        return pltpu.make_async_copy(src, dst, sems.at[_SEM[name] + i])

    def modw(i, rows):
        return jnp.concatenate([mod_v[:, i * D:(i + 1) * D]] * (rows // 8), axis=0)

    def mod(i):
        return mod_v[0:1, i * D:(i + 1) * D]

    c_cp = cp("c", c_hbm, c_v)
    def wm_cp(i):
        return cp("wm4", wm_hbm.at[:, _blk(i, 512)], wm_v.at[:, _blk(i, 512)], i)
    def wm2_cp(j):
        return cp("wn0", wm_hbm.at[:, _blk(4 + j, 512)], wm_v.at[:, _blk(4 + j, 512)], j)
    def x_cp(i):
        return cp("x0", x_hbm.at[_blk(min(i, NX - 1) if isinstance(i, int) else jnp.minimum(i, NX - 1), XC), :],
                  x_v.at[_blk(i, XC), :], i)
    def wq_cps(j):
        return [cp("wq0", wq_hbm.at[:, _blk(j * 4 + t, DH)], wq_v.at[j * 4 + t], j) for t in range(4)]
    wo_cps = [cp("wo", wo_hbm.at[:, pl.ds(n * 128, 128)], wo_v.at[n]) for n in range(D // 128)]
    wr_cp = cp("wr", wr_hbm, wr_v)
    wg_cp = cp("wg", wg_hbm, wg_v)
    wu_cp = cp("wu", wu_hbm, wu_v)
    wd_cp = cp("wd", wd_hbm, wd_v)
    out4 = out_hbm.reshape(NM, 8, RG, D)

    def out_cps(half):
        js = pl.ds(0, NM // 2 - 1) if half == 0 else pl.ds(NM // 2 - 1, NM // 2 + 1)
        return [cp("o0", piece[p].at[js, :, pl.ds(D, D)], out4.at[js, p], half * 8 + p) for p in range(8)]

    def kv_cps(grp, slot):
        heads = pl.ds(grp * G, G)
        return (cp("k0", k_hbm.at[heads], k_v.at[slot], slot), cp("v0", v_hbm.at[heads], v_v.at[slot], slot))

    c_cp.start()
    for i in range(4):
        wm_cp(i).start()
    x_cp(0).start()
    for c_ in wq_cps(0):
        c_.start()
    x_cp(1).start()

    for p_ in hbuf:
        p_[D // 128, 0:16, :] = jnp.zeros((16, 128), BF16)
    for p_ in piece:
        p_[NM, :, 0:128] = jnp.zeros((RG, 128), BF16)
    c_cp.wait()
    cf = c_v[...].astype(F32)
    sc = jnp.broadcast_to(cf * jax.nn.sigmoid(cf), (16, D)).astype(BF16)
    scb_v[...] = jnp.broadcast_to(sc[0:1].astype(F32), (128, D)).T
    for m_ in mp:
        m_[7] = jnp.zeros((8, 128), F32)

    def mod_body(i, carry):
        wm_cp(i).wait()
        mod_v[:, _blk(i, 512)] = jnp.dot(sc, wm_v[:, _blk(i, 512)], preferred_element_type=F32)[:8]
        return carry

    lax.fori_loop(0, 4, mod_body, 0)

    def ln1(i, p, dst, row0):
        rows = pl.ds(pl.multiple_of(i * XC + p * HG, HG), HG)
        xn = _layernorm(x_v[rows, :].astype(F32))
        for t in range(D // 128):
            dst[t, row0:row0 + HG, :] = (xn[:, t * 128:(t + 1) * 128] * modt(1, t, HG) + modt(0, t, HG)).astype(BF16)

    mod_v[:, D:2 * D] = 1.0 + mod_v[:, D:2 * D]
    x_cp(0).wait()
    for p in range(NH):
        ln1(0, p, hbuf[p], 0)
    for c_ in wq_cps(0):
        c_.wait()
    for i in range(2, NX + 1):
        x_cp(i).start()
    wm2_cp(0).start()
    for j_ in range(1, 8):
        for c_ in wq_cps(j_):
            c_.start()
        wm2_cp(j_).start()

    def p1a_body(i, carry):
        nxt = i + 1
        x_cp(nxt).wait()
        hv = [h.at[:, pl.ds(pl.multiple_of(i * HG, HG), 2 * HG), :] for h in hbuf]
        pos = 0
        for n in range(N0 // 128):
            for hf in range(2):
                wt = [wq_v[n, t * 128:(t + 1) * 128, :] for t in range(D // 128)]
                for half_ in range(2):
                    for c_, p in enumerate(LN_PIECES.get(pos, ())):
                        ln1(nxt, p, hv[p], HG)
                        t = 4 * half_ + c_
                        wt[t] = jnp.concatenate([after(wq_v[n, t * 128:t * 128 + 16, :], hbuf[p][D // 128, 0:16, :]),
                                                 wq_v[n, t * 128 + 16:(t + 1) * 128, :]], axis=0)
                    pos += 1
                lhs = jnp.concatenate(
                    [jnp.concatenate([hv[p][t, 0:HG, :] for t in range(D // 128)], axis=1)
                     for p in range(hf * NH // 2, (hf + 1) * NH // 2)], axis=0)
                q = jnp.dot(lhs, jnp.concatenate(wt, axis=0), preferred_element_type=F32)
                q_v[n, pl.ds(pl.multiple_of(i * XC + hf * (XC // 2), XC // 2), XC // 2), :] = (q * QSCALE).astype(BF16)
        return carry

    lax.fori_loop(0, NX, p1a_body, 0)

    for c_ in kv_cps(0, 0):
        c_.start()
    for c_ in (wr_cp, *wo_cps, wg_cp, wu_cp, wd_cp):
        c_.start()

    wm2_cp(0).wait()

    def p1b_body(j, carry):
        for c_ in wq_cps(j):
            c_.wait()
        wm2_cp(j).wait()
        tile0 = jnp.minimum(MT * (j - 1), 32 - MT)
        for r in range(S // 512):
            wt = [[wq_v[j * 4 + t, k * 128:(k + 1) * 128, :] for k in range(D // 128)] for t in range(4)]
            for p, k in MOD_PIECES.get(r, ()):
                wm = wm_v[:, pl.ds(pl.multiple_of(2 * D + (tile0 + p) * 128, 128), 128)].astype(F32)
                mp[p][j - 1] = jnp.broadcast_to(jnp.sum(wm * scb_v[...], axis=0, keepdims=True), (8, 128))
                z = jnp.concatenate([mp[p][7]] * 2, axis=0)
                wt[0][k] = jnp.concatenate([after(wq_v[j * 4, k * 128:k * 128 + 16, :], z),
                                            wq_v[j * 4, k * 128 + 16:(k + 1) * 128, :]], axis=0)
            w = jnp.concatenate([jnp.concatenate(c_, axis=0) for c_ in wt], axis=1)
            lhs = jnp.concatenate(
                [jnp.concatenate([hbuf[p][t, i * HG:(i + 1) * HG, :] for t in range(D // 128)], axis=1)
                 for i in (2 * r, 2 * r + 1) for p in range(NH)], axis=0)
            q = jnp.dot(lhs, w, preferred_element_type=F32) * QSCALE
            for t in range(4):
                q_v[j * 4 + t, r * 512:(r + 1) * 512, :] = q[:, t * DH:(t + 1) * DH].astype(BF16)
        return carry

    lax.fori_loop(1, 8, p1b_body, 0)
    for c_ in range(32):
        j_ = min(c_ // MT, 6)
        mod_v[:, 2 * D + c_ * 128:2 * D + (c_ + 1) * 128] = mp[c_ - min(MT * j_, 32 - MT)][j_]

    def p2_body(grp, carry):
        slot = grp % 2

        for c_ in kv_cps(jnp.minimum(grp + 1, H // G - 1), 1 - slot):
            c_.start()
        for c_ in kv_cps(grp, slot):
            c_.wait()
        for hh in range(G):
            head = grp * G + hh
            r0 = 0
            for nr in SUBS[hh]:
                rows = pl.ds(r0, nr)
                r0 += nr
                o_v[head, rows, :] = _attn(q_v[head, rows, :], k_v[slot, hh], v_v[slot, hh])
        return carry

    lax.fori_loop(0, H // G, p2_body, 0)
    for c_ in kv_cps(H // G - 1, (H // G) % 2):
        c_.wait()

    mod_v[:, 4 * D:5 * D] = (1.0 + mod_v[:, 4 * D:5 * D].astype(BF16).astype(F32)).astype(BF16).astype(F32)

    for c_ in wo_cps:
        c_.wait()
    wr_cp.wait()
    wr = wr_v[...].astype(F32)
    for t in range(D // 128):
        mod_v[:, t * 128:(t + 1) * 128] = jnp.broadcast_to(wr[t:t + 1, :], (8, 128))
    lane = lax.broadcasted_iota(jnp.int32, (8, 128), 1)
    acc_v[0] = jnp.zeros((MC, D), F32)

    def finish(j, p, acc):
        rows = pl.ds(pl.multiple_of(j * MC + p * RG, RG), RG)
        x2 = x_v[rows, :].astype(F32) + modw(2, RG) * acc[p * RG:(p + 1) * RG, :]
        h2 = (_layernorm(x2) * modw(4, RG) + modw(3, RG)).astype(BF16)
        piece[p][j, :, 0:D] = h2
        h2 = h2.astype(F32)
        piece[p][j, :, D:2 * D] = (x2 + modw(5, RG) * (h2 + h2 * 0.0)).astype(BF16)
        e = h2 * modw(0, RG)
        pr = None
        for t in range(D // 128):
            pr = e[:, t * 128:(t + 1) * 128] if pr is None else pr + e[:, t * 128:(t + 1) * 128]
        r = jnp.sum(pr, axis=1, keepdims=True)
        r_v[p] = jnp.where(lane == 2 * j, r[0:8], jnp.where(lane == 2 * j + 1, r[8:16], r_v[p]))
        return r

    def p3_body(j, carry):
        jp = jnp.maximum(j - 1, 0)
        accs = acc_v.at[pl.ds(j, 2)]
        for n in range(D // 128):
            cols = slice(n * 128, (n + 1) * 128)
            row0 = pl.multiple_of(j * MC, MC)
            tiles = [o_v[h, pl.ds(row0, MC), :] for h in range(H)]
            for p in PIECES.get(n, ()):
                r = finish(jp, p, accs.at[0])
                tiles[p] = jnp.concatenate([after(o_v[p, pl.ds(row0, 16), :], piece[p][NM, :, 0:128], r),
                                            o_v[p, pl.ds(row0 + 16, MC - 16), :]], axis=0)
            lhs = jnp.concatenate(tiles, axis=1)
            accs[1, :, cols] = jnp.dot(lhs, wo_v[n], preferred_element_type=F32)

        return carry

    def p3_half(half, carry):
        lax.fori_loop(half * (NM // 2), (half + 1) * (NM // 2), p3_body, 0)

        @pl.when(half == 0)
        def _():
            for c_ in out_cps(0):
                c_.start()
        return carry

    r_v[...] = jnp.zeros_like(r_v)
    lax.fori_loop(0, 2, p3_half, 0)
    for p in range(8):
        finish(NM - 1, p, acc_v.at[NM])

    r = r_v[...].astype(BF16).astype(F32)
    ln_ = lax.broadcasted_iota(jnp.int32, r.shape, 2)
    tok = (lax.broadcasted_iota(jnp.int32, r.shape, 0) * RG + (ln_ // 2) * MC + (ln_ % 2) * 8
           + lax.broadcasted_iota(jnp.int32, r.shape, 1))
    valid = ln_ < 2 * NM
    tokf = tok.astype(F32)

    def top1(cand):
        rr = jnp.where(cand, r, -jnp.inf)
        m = jnp.max(rr)
        i = jnp.min(jnp.where(cand & (rr == m), tokf, float(S)))
        return m, jnp.clip(i.astype(jnp.int32), 0, S - 1)

    m0, i0 = top1(valid)
    m1, i1 = top1(valid & (tok != i0))
    base = [pl.multiple_of((i // RG) * RG, RG) for i in (i0, i1)]
    for s_, b_ in enumerate(base):
        for p in range(8):
            @pl.when((b_ % MC) // RG == p)
            def _(s_=s_, b_=b_, p=p):
                sel_v[s_] = piece[p][b_ // MC]
    row16 = lax.broadcasted_iota(jnp.int32, (16, D), 0)
    won = [row16 + base[s_] == i_ for s_, i_ in enumerate((i0, i1))]
    xrow = [jnp.sum(jnp.where(won[s_], sel_v[s_, :, 0:D].astype(F32), 0.0), axis=0, keepdims=True) for s_ in range(2)]
    xs = jnp.where(row16 == 0, xrow[0], jnp.where(row16 == 1, xrow[1], 0.0)).astype(BF16)

    for c_ in out_cps(1):
        c_.start()
    wg_cp.wait()
    wu_cp.wait()
    wd_cp.wait()

    y = None
    for f in range(FF // FB):
        cols = slice(f * FB, (f + 1) * FB)
        g = jnp.dot(xs, wg_v[:, cols], preferred_element_type=F32)
        u = jnp.dot(xs, wu_v[:, cols], preferred_element_type=F32)
        act = (g * jax.nn.sigmoid(g) * u).astype(BF16)
        d = jnp.dot(act, wd_v[cols, :], preferred_element_type=F32)
        y = d if y is None else y + d
    y0 = y[0:1] * jax.nn.sigmoid(jnp.full((1, D), m0, F32))
    y1 = y[1:2] * jax.nn.sigmoid(jnp.full((1, D), m1, F32))
    for s_ in range(2):
        upd = jnp.where(row16 + base[s_] == i0, y0, jnp.where(row16 + base[s_] == i1, y1, 0.0))
        fix_v[s_] = (sel_v[s_, :, D:2 * D].astype(F32) + mod(5) * upd).astype(BF16)

    for c_ in out_cps(0) + out_cps(1):
        c_.wait()
    fix = [cp("f0", fix_v.at[s_], out_hbm.at[pl.ds(base[s_], 16), :], s_) for s_ in range(2)]
    fix[0].start()

    @pl.when(base[0] != base[1])
    def _():
        fix[1].start()
        fix[1].wait()

    fix[0].wait()


@jax.jit
def pallas_adaLN_cond__mha_block_cached__moe_arch_mod__prompt_kernel(
    A_x: jax.Array,
    A_k_cache: jax.Array,
    A_v_cache: jax.Array,
    A_wq: jax.Array,
    A_wo: jax.Array,
    B_x: jax.Array,
    B_w_r: jax.Array,
    B_w_gate: jax.Array,
    B_w_up: jax.Array,
    B_w_down: jax.Array,
    c: jax.Array,
    w_mod: jax.Array,
):
    any_spec = pl.BlockSpec(memory_space=pl.ANY)
    vm = pltpu.VMEM
    out = pl.pallas_call(
        _kernel,
        name="adaln_mha_moe",
        in_specs=[any_spec] * 11,
        out_specs=any_spec,
        out_shape=jax.ShapeDtypeStruct((S, D), BF16),
        scratch_shapes=[
            vm((S + XC, D), BF16),
            vm((H, D, DH), BF16),
            vm((H, S, DH), BF16),
            vm((H, S, DH), BF16),
            vm((2, G, S, DH), BF16),
            vm((2, G, S, DH), BF16),
            vm((D // 128, H * DH, 128), BF16),
            vm((8, 128), BF16),
            vm((D, FF), BF16),
            vm((D, FF), BF16),
            vm((FF, D), BF16),
            vm((1, D), BF16),
            vm((D, 6 * D), BF16),
            vm((8, 6 * D), F32),
            vm((D, 128), F32),
            vm((NM + 1, MC, D), F32),
            vm((8, 8, 128), F32),
            vm((2, RG, 2 * D), BF16),
            vm((2, 16, D), BF16),
            pltpu.SemaphoreType.DMA((len(_names),)),
            *[vm((D // 128 + 1, (NX + 1) * HG, 128), BF16)] * NH,
            *[vm((NM + 1, RG, 2 * D), BF16)] * 8,
            *[vm((8, 8, 128), F32)] * MT,
        ],
        compiler_params=pltpu.CompilerParams(vmem_limit_bytes=124 * 1024 * 1024),
    )(
        A_x.reshape(S, D), A_k_cache.reshape(H, S, DH), A_v_cache.reshape(H, S, DH), A_wq, A_wo,
        B_w_r.reshape(8, 128), B_w_gate, B_w_up, B_w_down, c, w_mod,
    )
    return out.reshape(1, S, D)
```

```python
import functools
import math

import jax
import jax.numpy as jnp
from jax import lax
from jax.experimental import pallas as pl
from jax.experimental.pallas import tpu as pltpu

F32 = jnp.float32
BF16 = jnp.bfloat16

S = 2048
D = 1024
H = 32
DH = 128
FF = 3584
EPS = 1e-5
QSCALE = (DH ** -0.5) * math.log2(math.e)

G = 2
SUBS = ((256, 384, 384, 512, 512), (512, 512, 384, 384, 256))
N0 = 512
N1 = 512
XC = 256
NX = S // XC
NH = 16
HG = XC // NH
MC = 128
NM = S // MC
RG = MC // 8
PIECES = {1: [0], 2: [1], 3: [2], 4: [3], 5: [4], 6: [5], 7: [6, 7]}
LN_PIECES = {3: [0], 4: [1], 5: [2], 6: [3], 7: [4], 8: [5], 9: [6], 10: [7], 11: [8], 12: [9], 13: [10, 11], 14: [12, 13], 15: [14, 15]}
MOD_PIECES = {0: [(0, 4)], 1: [(1, 0), (2, 4)], 2: [(3, 0), (4, 4)]}
MT = 5
FB = 512
NT = (((1,), (1,)), ((), ()))

_names = (["c", "wr", "wg", "wu", "wd", "wo", "f0", "f1"]
          + ["wq%d" % i for i in range(8)] + ["wn%d" % i for i in range(8)] + ["wm%d" % i for i in range(4, 8)] + ["x%d" % i for i in range(NX + 1)]
          + ["k0", "k1", "v0", "v1"] + ["o%d" % i for i in range(NM)])
_SEM = {n: i for i, n in enumerate(_names)}


def _attn(q, k, v):
    s = lax.dot_general(q, k, NT, preferred_element_type=F32)
    m = jnp.max(s, axis=1, keepdims=True)
    p = jnp.exp2(s - m)
    grp = 4
    acc = None
    tiles = []
    for g in range(S // (128 * grp)):
        ts = [p[:, (g * grp + j) * 128:(g * grp + j + 1) * 128] for j in range(grp)]
        t = (ts[0] + ts[1]) + (ts[2] + ts[3])
        acc = t if acc is None else acc + t
        tiles += ts[:-1] + [jnp.minimum(ts[-1], acc)]
    l = jnp.sum(acc, axis=1, keepdims=True)
    o = jnp.dot(jnp.concatenate(tiles, axis=1).astype(BF16), v, preferred_element_type=F32)
    return (o * pl.reciprocal(l, approx=True)).astype(BF16)


def _layernorm(x):
    xc = x - jnp.mean(x, axis=1, keepdims=True)
    var = jnp.mean(xc * xc, axis=1, keepdims=True)
    return xc * lax.rsqrt(var + EPS)


def _blk(i, n):
    return pl.ds(i * n if isinstance(i, int) else pl.multiple_of(i * n, n), n)


def _kernel(x_hbm, k_hbm, v_hbm, wq_hbm, wo_hbm, wr_hbm, wg_hbm, wu_hbm, wd_hbm,
            c_hbm, wm_hbm, out_hbm,
            x_v, wq_v, q_v, o_v, k_v, v_v, wo_v, wr_v, wg_v, wu_v, wd_v, c_v,
            wm_v, mod_v, scb_v, acc_v, r_v, sel_v, fix_v, sems, *bufs):

    piece = bufs[NH:NH + 8]
    mp = bufs[NH + 8:]

    def after(t, z, r=None):
        z = z.astype(F32)
        if r is not None:
            z = lax.bitcast_convert_type(
                lax.bitcast_convert_type(z, jnp.int32)
                & lax.bitcast_convert_type(jnp.broadcast_to(r, z.shape), jnp.int32), F32)
        return (t.astype(F32) + z).astype(BF16)

    def modt(i, t, rows):
        m = mod_v[:, i * D + t * 128:i * D + (t + 1) * 128]
        return jnp.concatenate([m] * (rows // 8), axis=0)

    hbuf = bufs[:NH]

    def cp(name, src, dst, i=0):
        return pltpu.make_async_copy(src, dst, sems.at[_SEM[name] + i])

    def modw(i, rows):
        return jnp.concatenate([mod_v[:, i * D:(i + 1) * D]] * (rows // 8), axis=0)

    def mod(i):
        return mod_v[0:1, i * D:(i + 1) * D]

    c_cp = cp("c", c_hbm, c_v)
    def wm_cp(i):
        return cp("wm4", wm_hbm.at[:, _blk(i, 512)], wm_v.at[:, _blk(i, 512)], i)
    def wm2_cp(j):
        return cp("wn0", wm_hbm.at[:, _blk(4 + j, 512)], wm_v.at[:, _blk(4 + j, 512)], j)
    def x_cp(i):
        return cp("x0", x_hbm.at[_blk(min(i, NX - 1) if isinstance(i, int) else jnp.minimum(i, NX - 1), XC), :],
                  x_v.at[_blk(i, XC), :], i)
    def wq_cps(j):
        return [cp("wq0", wq_hbm.at[:, _blk(j * 4 + t, DH)], wq_v.at[j * 4 + t], j) for t in range(4)]
    wo_cps = [cp("wo", wo_hbm.at[:, pl.ds(n * 128, 128)], wo_v.at[n]) for n in range(D // 128)]
    wr_cp = cp("wr", wr_hbm, wr_v)
    wg_cp = cp("wg", wg_hbm, wg_v)
    wu_cp = cp("wu", wu_hbm, wu_v)
    wd_cp = cp("wd", wd_hbm, wd_v)
    out4 = out_hbm.reshape(NM, 8, RG, D)

    def out_cps(half):
        js = pl.ds(0, NM // 2 - 1) if half == 0 else pl.ds(NM // 2 - 1, NM // 2 + 1)
        return [cp("o0", piece[p].at[js, :, pl.ds(D, D)], out4.at[js, p], half * 8 + p) for p in range(8)]

    def kv_cps(grp, slot):
        heads = pl.ds(grp * G, G)
        return (cp("k0", k_hbm.at[heads], k_v.at[slot], slot), cp("v0", v_hbm.at[heads], v_v.at[slot], slot))

    c_cp.start()
    for i in range(4):
        wm_cp(i).start()
    x_cp(0).start()
    for c_ in wq_cps(0):
        c_.start()
    x_cp(1).start()

    for p_ in hbuf:
        p_[D // 128, 0:16, :] = jnp.zeros((16, 128), BF16)
    for p_ in piece:
        p_[NM, :, 0:128] = jnp.zeros((RG, 128), BF16)
    c_cp.wait()
    cf = c_v[...].astype(F32)
    sc = jnp.broadcast_to(cf * jax.nn.sigmoid(cf), (16, D)).astype(BF16)
    scb_v[...] = jnp.broadcast_to(sc[0:1].astype(F32), (128, D)).T
    for m_ in mp:
        m_[7] = jnp.zeros((8, 128), F32)

    def mod_body(i, carry):
        wm_cp(i).wait()
        mod_v[:, _blk(i, 512)] = jnp.dot(sc, wm_v[:, _blk(i, 512)], preferred_element_type=F32)[:8]
        return carry

    lax.fori_loop(0, 4, mod_body, 0)

    def ln1(i, p, dst, row0):
        rows = pl.ds(pl.multiple_of(i * XC + p * HG, HG), HG)
        xn = _layernorm(x_v[rows, :].astype(F32))
        for t in range(D // 128):
            dst[t, row0:row0 + HG, :] = (xn[:, t * 128:(t + 1) * 128] * modt(1, t, HG) + modt(0, t, HG)).astype(BF16)

    mod_v[:, D:2 * D] = 1.0 + mod_v[:, D:2 * D]
    x_cp(0).wait()
    for p in range(NH):
        ln1(0, p, hbuf[p], 0)
    for c_ in wq_cps(0):
        c_.wait()
    for i in range(2, NX + 1):
        x_cp(i).start()
    wm2_cp(0).start()
    for j_ in range(1, 8):
        for c_ in wq_cps(j_):
            c_.start()
        wm2_cp(j_).start()

    def p1a_body(i, carry):
        nxt = i + 1
        x_cp(nxt).wait()
        hv = [h.at[:, pl.ds(pl.multiple_of(i * HG, HG), 2 * HG), :] for h in hbuf]
        pos = 0
        for n in range(N0 // 128):
            for hf in range(2):
                wt = [wq_v[n, t * 128:(t + 1) * 128, :] for t in range(D // 128)]
                for half_ in range(2):
                    for c_, p in enumerate(LN_PIECES.get(pos, ())):
                        ln1(nxt, p, hv[p], HG)
                        t = 4 * half_ + c_
                        wt[t] = jnp.concatenate([after(wq_v[n, t * 128:t * 128 + 16, :], hbuf[p][D // 128, 0:16, :]),
                                                 wq_v[n, t * 128 + 16:(t + 1) * 128, :]], axis=0)
                    pos += 1
                lhs = jnp.concatenate(
                    [jnp.concatenate([hv[p][t, 0:HG, :] for t in range(D // 128)], axis=1)
                     for p in range(hf * NH // 2, (hf + 1) * NH // 2)], axis=0)
                q = jnp.dot(lhs, jnp.concatenate(wt, axis=0), preferred_element_type=F32)
                q_v[n, pl.ds(pl.multiple_of(i * XC + hf * (XC // 2), XC // 2), XC // 2), :] = (q * QSCALE).astype(BF16)
        return carry

    lax.fori_loop(0, NX, p1a_body, 0)

    for c_ in kv_cps(0, 0):
        c_.start()
    for c_ in (wr_cp, *wo_cps, wg_cp, wu_cp, wd_cp):
        c_.start()

    wm2_cp(0).wait()

    def p1b_body(j, carry):
        for c_ in wq_cps(j):
            c_.wait()
        wm2_cp(j).wait()
        tile0 = jnp.minimum(MT * (j - 1), 32 - MT)
        for r in range(S // 512):
            wt = [[wq_v[j * 4 + t, k * 128:(k + 1) * 128, :] for k in range(D // 128)] for t in range(4)]
            for p, k in MOD_PIECES.get(r, ()):
                wm = wm_v[:, pl.ds(pl.multiple_of(2 * D + (tile0 + p) * 128, 128), 128)].astype(F32)
                mp[p][j - 1] = jnp.broadcast_to(jnp.sum(wm * scb_v[...], axis=0, keepdims=True), (8, 128))
                z = jnp.concatenate([mp[p][7]] * 2, axis=0)
                wt[0][k] = jnp.concatenate([after(wq_v[j * 4, k * 128:k * 128 + 16, :], z),
                                            wq_v[j * 4, k * 128 + 16:(k + 1) * 128, :]], axis=0)
            w = jnp.concatenate([jnp.concatenate(c_, axis=0) for c_ in wt], axis=1)
            lhs = jnp.concatenate(
                [jnp.concatenate([hbuf[p][t, i * HG:(i + 1) * HG, :] for t in range(D // 128)], axis=1)
                 for i in (2 * r, 2 * r + 1) for p in range(NH)], axis=0)
            q = jnp.dot(lhs, w, preferred_element_type=F32) * QSCALE
            for t in range(4):
                q_v[j * 4 + t, r * 512:(r + 1) * 512, :] = q[:, t * DH:(t + 1) * DH].astype(BF16)
        return carry

    lax.fori_loop(1, 8, p1b_body, 0)
    for c_ in range(32):
        j_ = min(c_ // MT, 6)
        mod_v[:, 2 * D + c_ * 128:2 * D + (c_ + 1) * 128] = mp[c_ - min(MT * j_, 32 - MT)][j_]

    def p2_body(grp, carry):
        slot = grp % 2

        for c_ in kv_cps(jnp.minimum(grp + 1, H // G - 1), 1 - slot):
            c_.start()
        for c_ in kv_cps(grp, slot):
            c_.wait()
        for hh in range(G):
            head = grp * G + hh
            r0 = 0
            for nr in SUBS[hh]:
                rows = pl.ds(r0, nr)
                r0 += nr
                o_v[head, rows, :] = _attn(q_v[head, rows, :], k_v[slot, hh], v_v[slot, hh])
        return carry

    lax.fori_loop(0, H // G, p2_body, 0)
    for c_ in kv_cps(H // G - 1, (H // G) % 2):
        c_.wait()

    mod_v[:, 4 * D:5 * D] = (1.0 + mod_v[:, 4 * D:5 * D].astype(BF16).astype(F32)).astype(BF16).astype(F32)

    for c_ in wo_cps:
        c_.wait()
    wr_cp.wait()
    wr = wr_v[...].astype(F32)
    for t in range(D // 128):
        mod_v[:, t * 128:(t + 1) * 128] = jnp.broadcast_to(wr[t:t + 1, :], (8, 128))
    lane = lax.broadcasted_iota(jnp.int32, (8, 128), 1)
    acc_v[0] = jnp.zeros((MC, D), F32)

    def finish(j, p, acc):
        rows = pl.ds(pl.multiple_of(j * MC + p * RG, RG), RG)
        x2 = x_v[rows, :].astype(F32) + modw(2, RG) * acc[p * RG:(p + 1) * RG, :]
        h2 = (_layernorm(x2) * modw(4, RG) + modw(3, RG)).astype(BF16)
        piece[p][j, :, 0:D] = h2
        h2 = h2.astype(F32)
        piece[p][j, :, D:2 * D] = (x2 + modw(5, RG) * (h2 + h2 * 0.0)).astype(BF16)
        e = h2 * modw(0, RG)
        pr = None
        for t in range(D // 128):
            pr = e[:, t * 128:(t + 1) * 128] if pr is None else pr + e[:, t * 128:(t + 1) * 128]
        r = jnp.sum(pr, axis=1, keepdims=True)
        r_v[p] = jnp.where(lane == 2 * j, r[0:8], jnp.where(lane == 2 * j + 1, r[8:16], r_v[p]))
        return r

    def p3_body(j, carry):
        jp = jnp.maximum(j - 1, 0)
        accs = acc_v.at[pl.ds(j, 2)]
        for n in range(D // 128):
            cols = slice(n * 128, (n + 1) * 128)
            row0 = pl.multiple_of(j * MC, MC)
            tiles = [o_v[h, pl.ds(row0, MC), :] for h in range(H)]
            for p in PIECES.get(n, ()):
                r = finish(jp, p, accs.at[0])
                tiles[p] = jnp.concatenate([after(o_v[p, pl.ds(row0, 16), :], piece[p][NM, :, 0:128], r),
                                            o_v[p, pl.ds(row0 + 16, MC - 16), :]], axis=0)
            lhs = jnp.concatenate(tiles, axis=1)
            accs[1, :, cols] = jnp.dot(lhs, wo_v[n], preferred_element_type=F32)

        return carry

    def p3_half(half, carry):
        lax.fori_loop(half * (NM // 2), (half + 1) * (NM // 2), p3_body, 0)

        @pl.when(half == 0)
        def _():
            for c_ in out_cps(0):
                c_.start()
        return carry

    r_v[...] = jnp.zeros_like(r_v)
    lax.fori_loop(0, 2, p3_half, 0)
    for p in range(8):
        finish(NM - 1, p, acc_v.at[NM])

    r = r_v[...].astype(BF16).astype(F32) + 0.0
    ln_ = lax.broadcasted_iota(jnp.int32, r.shape, 2)
    tok = (lax.broadcasted_iota(jnp.int32, r.shape, 0) * RG + (ln_ // 2) * MC + (ln_ % 2) * 8
           + lax.broadcasted_iota(jnp.int32, r.shape, 1))
    u = lax.shift_right_logical(lax.bitcast_convert_type(r, jnp.int32), 16)
    u = jnp.where(u >= 0x8000, 0xFFFF - u, u + 0x8000)
    key = jnp.where(ln_ < 2 * NM, (u << 11) + (S - 1 - tok) + (1 << 27), 0)
    key = lax.bitcast_convert_type(key, F32)

    def top1(k):
        m = jnp.max(jnp.max(k, axis=0), axis=0, keepdims=True)
        m = jnp.max(m, axis=1, keepdims=True)
        bits = lax.bitcast_convert_type(m, jnp.int32)
        u_ = (bits >> 11) & 0xFFFF
        u_ = jnp.where(u_ >= 0x8000, u_ - 0x8000, 0xFFFF - u_)
        score = lax.bitcast_convert_type(u_ << 16, F32)
        return m, (S - 1) - (bits & (S - 1))[0, 0], jax.nn.sigmoid(score)

    m0, i0, g0 = top1(key)
    m1, i1, g1 = top1(jnp.where(key == m0, 0.0, key))
    base = [pl.multiple_of((i // RG) * RG, RG) for i in (i0, i1)]
    for s_, b_ in enumerate(base):
        for p in range(8):
            @pl.when((b_ % MC) // RG == p)
            def _(s_=s_, b_=b_, p=p):
                sel_v[s_] = piece[p][b_ // MC]
    row16 = lax.broadcasted_iota(jnp.int32, (16, D), 0)
    won = [row16 + base[s_] == i_ for s_, i_ in enumerate((i0, i1))]
    xrow = [jnp.sum(jnp.where(won[s_], sel_v[s_, :, 0:D].astype(F32), 0.0), axis=0, keepdims=True) for s_ in range(2)]
    xs = jnp.where(row16 == 0, xrow[0], jnp.where(row16 == 1, xrow[1], 0.0)).astype(BF16)

    for c_ in out_cps(1):
        c_.start()
    wg_cp.wait()
    wu_cp.wait()
    wd_cp.wait()

    y = None
    for f in range(FF // FB):
        cols = slice(f * FB, (f + 1) * FB)
        g = jnp.dot(xs, wg_v[:, cols], preferred_element_type=F32)
        u = jnp.dot(xs, wu_v[:, cols], preferred_element_type=F32)
        act = (g * jax.nn.sigmoid(g) * u).astype(BF16)
        d = jnp.dot(act, wd_v[cols, :], preferred_element_type=F32)
        y = d if y is None else y + d
    y0 = y[0:1] * g0
    y1 = y[1:2] * g1
    for s_ in range(2):
        upd = jnp.where(row16 + base[s_] == i0, y0, jnp.where(row16 + base[s_] == i1, y1, 0.0))
        fix_v[s_] = (sel_v[s_, :, D:2 * D].astype(F32) + mod(5) * upd).astype(BF16)

    for c_ in out_cps(0) + out_cps(1):
        c_.wait()
    fix = [cp("f0", fix_v.at[s_], out_hbm.at[pl.ds(base[s_], 16), :], s_) for s_ in range(2)]
    fix[0].start()

    @pl.when(base[0] != base[1])
    def _():
        fix[1].start()
        fix[1].wait()

    fix[0].wait()


@jax.jit
def pallas_adaLN_cond__mha_block_cached__moe_arch_mod__prompt_kernel(
    A_x: jax.Array,
    A_k_cache: jax.Array,
    A_v_cache: jax.Array,
    A_wq: jax.Array,
    A_wo: jax.Array,
    B_x: jax.Array,
    B_w_r: jax.Array,
    B_w_gate: jax.Array,
    B_w_up: jax.Array,
    B_w_down: jax.Array,
    c: jax.Array,
    w_mod: jax.Array,
):
    any_spec = pl.BlockSpec(memory_space=pl.ANY)
    vm = pltpu.VMEM
    out = pl.pallas_call(
        _kernel,
        name="adaln_mha_moe",
        in_specs=[any_spec] * 11,
        out_specs=any_spec,
        out_shape=jax.ShapeDtypeStruct((S, D), BF16),
        scratch_shapes=[
            vm((S + XC, D), BF16),
            vm((H, D, DH), BF16),
            vm((H, S, DH), BF16),
            vm((H, S, DH), BF16),
            vm((2, G, S, DH), BF16),
            vm((2, G, S, DH), BF16),
            vm((D // 128, H * DH, 128), BF16),
            vm((8, 128), BF16),
            vm((D, FF), BF16),
            vm((D, FF), BF16),
            vm((FF, D), BF16),
            vm((1, D), BF16),
            vm((D, 6 * D), BF16),
            vm((8, 6 * D), F32),
            vm((D, 128), F32),
            vm((NM + 1, MC, D), F32),
            vm((8, 8, 128), F32),
            vm((2, RG, 2 * D), BF16),
            vm((2, 16, D), BF16),
            pltpu.SemaphoreType.DMA((len(_names),)),
            *[vm((D // 128 + 1, (NX + 1) * HG, 128), BF16)] * NH,
            *[vm((NM + 1, RG, 2 * D), BF16)] * 8,
            *[vm((8, 8, 128), F32)] * MT,
        ],
        compiler_params=pltpu.CompilerParams(vmem_limit_bytes=124 * 1024 * 1024),
    )(
        A_x.reshape(S, D), A_k_cache.reshape(H, S, DH), A_v_cache.reshape(H, S, DH), A_wq, A_wo,
        B_w_r.reshape(8, 128), B_w_gate, B_w_up, B_w_down, c, w_mod,
    )
    return out.reshape(1, S, D)
```

```python
import functools
import math

import jax
import jax.numpy as jnp
from jax import lax
from jax.experimental import pallas as pl
from jax.experimental.pallas import tpu as pltpu

F32 = jnp.float32
BF16 = jnp.bfloat16
U32 = jnp.uint32

S = 2048
D = 1024
H = 32
DH = 128
FF = 3584
EPS = 1e-5
QSCALE = (DH ** -0.5) * math.log2(math.e)

G = 2
SUBS = ((256, 384, 384, 512, 512), (512, 512, 384, 384, 256))
N0 = 512
N1 = 512
XC = 256
NX = S // XC
NH = 16
HG = XC // NH
MC = 128
NM = S // MC
RG = MC // 8
PIECES = {1: [0], 2: [1], 3: [2], 4: [3], 5: [4], 6: [5], 7: [6, 7]}
LN_PIECES = {2: [0], 3: [1], 4: [2], 5: [3], 6: [4], 7: [5], 8: [6], 9: [7], 10: [8], 11: [9], 12: [10], 13: [11], 14: [12], 15: [13, 14, 15]}
MOD_PIECES = {0: [(0, 4)], 1: [(1, 0), (2, 4)], 2: [(3, 0), (4, 4)]}
MT = 5
FB = 512
NT = (((1,), (1,)), ((), ()))

_names = (["c", "wr", "wg", "wu", "wd", "wo", "f0", "f1"]
          + ["wq%d" % i for i in range(8)] + ["wn%d" % i for i in range(8)] + ["wm%d" % i for i in range(4, 8)] + ["x%d" % i for i in range(NX + 1)]
          + ["k0", "k1", "v0", "v1"] + ["o%d" % i for i in range(NM)])
_SEM = {n: i for i, n in enumerate(_names)}


def _attn(q, k, v):
    s = lax.dot_general(q, k, NT, preferred_element_type=F32)
    m = jnp.max(s, axis=1, keepdims=True)
    p = jnp.exp2(s - m)
    grp = 4
    acc = None
    tiles = []
    for g in range(S // (128 * grp)):
        ts = [p[:, (g * grp + j) * 128:(g * grp + j + 1) * 128] for j in range(grp)]
        t = (ts[0] + ts[1]) + (ts[2] + ts[3])
        acc = t if acc is None else acc + t
        tiles += ts[:-1] + [jnp.minimum(ts[-1], acc)]
    l = jnp.sum(acc, axis=1, keepdims=True)
    o = jnp.dot(jnp.concatenate(tiles, axis=1).astype(BF16), v, preferred_element_type=F32)
    return (o * pl.reciprocal(l, approx=True)).astype(BF16)


def _layernorm(x):
    xc = x - jnp.mean(x, axis=1, keepdims=True)
    var = jnp.mean(xc * xc, axis=1, keepdims=True)
    return xc * lax.rsqrt(var + EPS)


def _blk(i, n):
    return pl.ds(i * n if isinstance(i, int) else pl.multiple_of(i * n, n), n)


def _half(r0):
    return r0 // 2 if isinstance(r0, int) else pl.multiple_of(r0 // 2, 8)


def _ld(ref, lead, r0=0, n=None):
    n = ref.shape[-2] - r0 if n is None else n
    return pltpu.bitcast(ref.bitcast(U32)[(*lead, pl.ds(_half(r0), n // 2), slice(None))], BF16)


def _kernel(x_hbm, k_hbm, v_hbm, wq_hbm, wo_hbm, wr_hbm, wg_hbm, wu_hbm, wd_hbm,
            c_hbm, wm_hbm, out_hbm,
            x_v, wq_v, q_v, o_v, k_v, v_v, wo_v, wr_v, wg_v, wu_v, wd_v, c_v,
            wm_v, mod_v, scb_v, acc_v, r_v, sel_v, fix_v, sems, *bufs):

    piece = bufs[NH:NH + 8]
    mp = bufs[NH + 8:]

    def after(t, z, r=None):
        z = pltpu.bitcast(z, U32)
        if r is not None:
            for r_ in (r[0:8], r[8:16]):
                z = z & lax.bitcast_convert_type(jnp.broadcast_to(r_, z.shape), U32)
        return pltpu.bitcast(pltpu.bitcast(t, U32) | z, BF16)

    def modt(i, t, rows):
        m = mod_v[:, i * D + t * 128:i * D + (t + 1) * 128]
        return jnp.concatenate([m] * (rows // 8), axis=0)

    hbuf = bufs[:NH]

    def cp(name, src, dst, i=0):
        return pltpu.make_async_copy(src, dst, sems.at[_SEM[name] + i])

    def modw(i, rows):
        return jnp.concatenate([mod_v[:, i * D:(i + 1) * D]] * (rows // 8), axis=0)

    def mod(i):
        return mod_v[0:1, i * D:(i + 1) * D]

    c_cp = cp("c", c_hbm, c_v)
    def wm_cp(i):
        return cp("wm4", wm_hbm.at[:, _blk(i, 512)], wm_v.at[:, _blk(i, 512)], i)
    def wm2_cp(j):
        return cp("wn0", wm_hbm.at[:, _blk(4 + j, 512)], wm_v.at[:, _blk(4 + j, 512)], j)
    def x_cp(i):
        return cp("x0", x_hbm.at[_blk(min(i, NX - 1) if isinstance(i, int) else jnp.minimum(i, NX - 1), XC), :],
                  x_v.at[_blk(i, XC), :], i)
    def wq_cps(j):
        return [cp("wq0", wq_hbm.at[:, _blk(j * 4 + t, DH)], wq_v.at[j * 4 + t], j) for t in range(4)]
    wo_cps = [cp("wo", wo_hbm.at[:, pl.ds(n * 128, 128)], wo_v.at[n]) for n in range(D // 128)]
    wr_cp = cp("wr", wr_hbm, wr_v)
    wg_cp = cp("wg", wg_hbm, wg_v)
    wu_cp = cp("wu", wu_hbm, wu_v)
    wd_cp = cp("wd", wd_hbm, wd_v)
    out4 = out_hbm.reshape(NM, 8, RG, D)

    def out_cps(half):
        js = pl.ds(0, NM // 2 - 1) if half == 0 else pl.ds(NM // 2 - 1, NM // 2 + 1)
        return [cp("o0", piece[p].at[js, :, pl.ds(D, D)], out4.at[js, p], half * 8 + p) for p in range(8)]

    def kv_cps(grp, slot):
        heads = pl.ds(grp * G, G)
        return (cp("k0", k_hbm.at[heads], k_v.at[slot], slot), cp("v0", v_hbm.at[heads], v_v.at[slot], slot))

    c_cp.start()
    for i in range(4):
        wm_cp(i).start()
    x_cp(0).start()
    for c_ in wq_cps(0):
        c_.start()
    x_cp(1).start()

    for p_ in hbuf:
        p_[D // 128, 0:16, :] = jnp.zeros((16, 128), BF16)
    for p_ in piece:
        p_[NM, :, 0:128] = jnp.zeros((RG, 128), BF16)
    c_cp.wait()
    cf = c_v[...].astype(F32)
    sc = jnp.broadcast_to(cf * jax.nn.sigmoid(cf), (16, D)).astype(BF16)
    scb_v[...] = jnp.broadcast_to(sc[0:1].astype(F32), (128, D)).T
    for m_ in mp:
        m_[7] = jnp.zeros((8, 128), F32)

    def mod_body(i, carry):
        wm_cp(i).wait()
        mod_v[:, _blk(i, 512)] = jnp.dot(sc, wm_v[:, _blk(i, 512)], preferred_element_type=F32)[:8]
        return carry

    lax.fori_loop(0, 4, mod_body, 0)

    def ln1(i, p, dst, row0):
        rows = pl.ds(pl.multiple_of(i * XC + p * HG, HG), HG)
        xn = _layernorm(x_v[rows, :].astype(F32))
        for t in range(D // 128):
            dst[t, row0:row0 + HG, :] = (xn[:, t * 128:(t + 1) * 128] * modt(1, t, HG) + modt(0, t, HG)).astype(BF16)

    mod_v[:, D:2 * D] = 1.0 + mod_v[:, D:2 * D]
    x_cp(0).wait()
    for p in range(NH):
        ln1(0, p, hbuf[p], 0)
    for c_ in wq_cps(0):
        c_.wait()
    for i in range(2, NX + 1):
        x_cp(i).start()
    wm2_cp(0).start()
    for j_ in range(1, 8):
        for c_ in wq_cps(j_):
            c_.start()
        wm2_cp(j_).start()

    def p1a_body(i, carry):
        nxt = i + 1
        x_cp(nxt).wait()
        hv = [h.at[:, pl.ds(pl.multiple_of(i * HG, HG), 2 * HG), :] for h in hbuf]
        pos = 0
        for n in range(N0 // 128):
            for hf in range(2):
                wt = [_ld(wq_v, (n,), t * 128, 128) for t in range(D // 128)]
                for half_ in range(2):
                    for c_, p in enumerate(LN_PIECES.get(pos, ())):
                        ln1(nxt, p, hv[p], HG)
                        t = 4 * half_ + c_
                        wt[t] = jnp.concatenate([after(_ld(wq_v, (n,), t * 128, 16), _ld(hbuf[p], (D // 128,), 0, 16)),
                                                 _ld(wq_v, (n,), t * 128 + 16, 112)], axis=0)
                    pos += 1
                lhs = jnp.concatenate(
                    [jnp.concatenate([_ld(hv[p], (t,), 0, HG) for t in range(D // 128)], axis=1)
                     for p in range(hf * NH // 2, (hf + 1) * NH // 2)], axis=0)
                q = jnp.dot(lhs, jnp.concatenate(wt, axis=0), preferred_element_type=F32)
                q_v[n, pl.ds(pl.multiple_of(i * XC + hf * (XC // 2), XC // 2), XC // 2), :] = (q * QSCALE).astype(BF16)
        return carry

    lax.fori_loop(0, NX, p1a_body, 0)

    for c_ in kv_cps(0, 0):
        c_.start()
    for c_ in (wr_cp, *wo_cps, wg_cp, wu_cp, wd_cp):
        c_.start()

    wm2_cp(0).wait()

    def p1b_body(j, carry):
        for c_ in wq_cps(j):
            c_.wait()
        wm2_cp(j).wait()
        tile0 = jnp.minimum(MT * (j - 1), 32 - MT)
        for r in range(S // 512):
            wt = [[_ld(wq_v, (j * 4 + t,), k * 128, 128) for k in range(D // 128)] for t in range(4)]
            for p, k in MOD_PIECES.get(r, ()):
                wm = wm_v[:, pl.ds(pl.multiple_of(2 * D + (tile0 + p) * 128, 128), 128)].astype(F32)
                mp[p][j - 1] = jnp.broadcast_to(jnp.sum(wm * scb_v[...], axis=0, keepdims=True), (8, 128))
                z = jnp.concatenate([mp[p][7]] * 2, axis=0)
                wt[0][k] = jnp.concatenate([after(_ld(wq_v, (j * 4,), k * 128, 16), z.astype(BF16)),
                                            _ld(wq_v, (j * 4,), k * 128 + 16, 112)], axis=0)
            w = jnp.concatenate([jnp.concatenate(c_, axis=0) for c_ in wt], axis=1)
            lhs = jnp.concatenate(
                [jnp.concatenate([_ld(hbuf[p], (t,), i * HG, HG) for t in range(D // 128)], axis=1)
                 for i in (2 * r, 2 * r + 1) for p in range(NH)], axis=0)
            q = jnp.dot(lhs, w, preferred_element_type=F32) * QSCALE
            for t in range(4):
                q_v[j * 4 + t, r * 512:(r + 1) * 512, :] = q[:, t * DH:(t + 1) * DH].astype(BF16)
        return carry

    lax.fori_loop(1, 8, p1b_body, 0)
    for c_ in range(32):
        j_ = min(c_ // MT, 6)
        mod_v[:, 2 * D + c_ * 128:2 * D + (c_ + 1) * 128] = mp[c_ - min(MT * j_, 32 - MT)][j_]

    def p2_body(grp, carry):
        slot = grp % 2

        for c_ in kv_cps(jnp.minimum(grp + 1, H // G - 1), 1 - slot):
            c_.start()
        for c_ in kv_cps(grp, slot):
            c_.wait()
        for hh in range(G):
            head = grp * G + hh
            r0 = 0
            for nr in SUBS[hh]:
                rows = pl.ds(r0, nr)
                r0 += nr
                o_v[head, rows, :] = _attn(q_v[head, rows, :], k_v[slot, hh], v_v[slot, hh])
        return carry

    lax.fori_loop(0, H // G, p2_body, 0)
    for c_ in kv_cps(H // G - 1, (H // G) % 2):
        c_.wait()

    mod_v[:, 4 * D:5 * D] = (1.0 + mod_v[:, 4 * D:5 * D].astype(BF16).astype(F32)).astype(BF16).astype(F32)

    for c_ in wo_cps:
        c_.wait()
    wr_cp.wait()
    wr = wr_v[...].astype(F32)
    for t in range(D // 128):
        mod_v[:, t * 128:(t + 1) * 128] = jnp.broadcast_to(wr[t:t + 1, :], (8, 128))
    lane = lax.broadcasted_iota(jnp.int32, (8, 128), 1)
    acc_v[0] = jnp.zeros((MC, D), F32)

    def finish(j, p, acc):
        rows = pl.ds(pl.multiple_of(j * MC + p * RG, RG), RG)
        x2 = x_v[rows, :].astype(F32) + modw(2, RG) * acc[p * RG:(p + 1) * RG, :]
        h2 = (_layernorm(x2) * modw(4, RG) + modw(3, RG)).astype(BF16)
        piece[p][j, :, 0:D] = h2
        h2 = h2.astype(F32)
        piece[p][j, :, D:2 * D] = (x2 + modw(5, RG) * (h2 + h2 * 0.0)).astype(BF16)
        e = h2 * modw(0, RG)
        pr = None
        for t in range(D // 128):
            pr = e[:, t * 128:(t + 1) * 128] if pr is None else pr + e[:, t * 128:(t + 1) * 128]
        r = jnp.sum(pr, axis=1, keepdims=True)
        r_v[p] = jnp.where(lane == 2 * j, r[0:8], jnp.where(lane == 2 * j + 1, r[8:16], r_v[p]))
        return r

    def p3_body(j, carry):
        jp = jnp.maximum(j - 1, 0)
        accs = acc_v.at[pl.ds(j, 2)]
        for n in range(D // 128):
            cols = slice(n * 128, (n + 1) * 128)
            row0 = pl.multiple_of(j * MC, MC)
            tiles = [_ld(o_v, (h,), row0, MC) for h in range(H)]
            for p in PIECES.get(n, ()):
                r = finish(jp, p, accs.at[0])
                tiles[p] = jnp.concatenate([after(_ld(o_v, (p,), row0, 16), piece[p][NM, :, 0:128], r),
                                            _ld(o_v, (p,), row0 + 16, MC - 16)], axis=0)
            lhs = jnp.concatenate(tiles, axis=1)
            accs[1, :, cols] = jnp.dot(lhs, _ld(wo_v, (n,)), preferred_element_type=F32)

        return carry

    def p3_half(half, carry):
        lax.fori_loop(half * (NM // 2), (half + 1) * (NM // 2), p3_body, 0)

        @pl.when(half == 0)
        def _():
            for c_ in out_cps(0):
                c_.start()
        return carry

    r_v[...] = jnp.zeros_like(r_v)
    lax.fori_loop(0, 2, p3_half, 0)
    for p in range(8):
        finish(NM - 1, p, acc_v.at[NM])

    r = r_v[...].astype(BF16).astype(F32) + 0.0
    ln_ = lax.broadcasted_iota(jnp.int32, r.shape, 2)
    tok = (lax.broadcasted_iota(jnp.int32, r.shape, 0) * RG + (ln_ // 2) * MC + (ln_ % 2) * 8
           + lax.broadcasted_iota(jnp.int32, r.shape, 1))
    u = lax.shift_right_logical(lax.bitcast_convert_type(r, jnp.int32), 16)
    u = jnp.where(u >= 0x8000, 0xFFFF - u, u + 0x8000)
    key = jnp.where(ln_ < 2 * NM, (u << 11) + (S - 1 - tok) + (1 << 27), 0)
    key = lax.bitcast_convert_type(key, F32)

    def top1(k):
        m = jnp.max(jnp.max(k, axis=0), axis=0, keepdims=True)
        m = jnp.max(m, axis=1, keepdims=True)
        bits = lax.bitcast_convert_type(m, jnp.int32)
        u_ = (bits >> 11) & 0xFFFF
        u_ = jnp.where(u_ >= 0x8000, u_ - 0x8000, 0xFFFF - u_)
        score = lax.bitcast_convert_type(u_ << 16, F32)
        return m, (S - 1) - (bits & (S - 1))[0, 0], jax.nn.sigmoid(score)

    m0, i0, g0 = top1(key)
    m1, i1, g1 = top1(jnp.where(key == m0, 0.0, key))
    base = [pl.multiple_of((i // RG) * RG, RG) for i in (i0, i1)]
    for s_, b_ in enumerate(base):
        for p in range(8):
            @pl.when((b_ % MC) // RG == p)
            def _(s_=s_, b_=b_, p=p):
                sel_v[s_] = piece[p][b_ // MC]
    row16 = lax.broadcasted_iota(jnp.int32, (16, D), 0)
    won = [row16 + base[s_] == i_ for s_, i_ in enumerate((i0, i1))]
    xrow = [jnp.sum(jnp.where(won[s_], sel_v[s_, :, 0:D].astype(F32), 0.0), axis=0, keepdims=True) for s_ in range(2)]
    xs = jnp.where(row16 == 0, xrow[0], jnp.where(row16 == 1, xrow[1], 0.0)).astype(BF16)

    for c_ in out_cps(1):
        c_.start()
    wg_cp.wait()
    wu_cp.wait()
    wd_cp.wait()

    y = None
    for f in range(FF // FB):
        cols = slice(f * FB, (f + 1) * FB)
        g = jnp.dot(xs, wg_v[:, cols], preferred_element_type=F32)
        u = jnp.dot(xs, wu_v[:, cols], preferred_element_type=F32)
        act = (g * jax.nn.sigmoid(g) * u).astype(BF16)
        d = jnp.dot(act, wd_v[cols, :], preferred_element_type=F32)
        y = d if y is None else y + d
    y0 = y[0:1] * g0
    y1 = y[1:2] * g1
    for s_ in range(2):
        upd = jnp.where(row16 + base[s_] == i0, y0, jnp.where(row16 + base[s_] == i1, y1, 0.0))
        fix_v[s_] = (sel_v[s_, :, D:2 * D].astype(F32) + mod(5) * upd).astype(BF16)

    for c_ in out_cps(0) + out_cps(1):
        c_.wait()
    fix = [cp("f0", fix_v.at[s_], out_hbm.at[pl.ds(base[s_], 16), :], s_) for s_ in range(2)]
    fix[0].start()

    @pl.when(base[0] != base[1])
    def _():
        fix[1].start()
        fix[1].wait()

    fix[0].wait()


@jax.jit
def pallas_adaLN_cond__mha_block_cached__moe_arch_mod__prompt_kernel(
    A_x: jax.Array,
    A_k_cache: jax.Array,
    A_v_cache: jax.Array,
    A_wq: jax.Array,
    A_wo: jax.Array,
    B_x: jax.Array,
    B_w_r: jax.Array,
    B_w_gate: jax.Array,
    B_w_up: jax.Array,
    B_w_down: jax.Array,
    c: jax.Array,
    w_mod: jax.Array,
):
    any_spec = pl.BlockSpec(memory_space=pl.ANY)
    vm = pltpu.VMEM
    out = pl.pallas_call(
        _kernel,
        name="adaln_mha_moe",
        in_specs=[any_spec] * 11,
        out_specs=any_spec,
        out_shape=jax.ShapeDtypeStruct((S, D), BF16),
        scratch_shapes=[
            vm((S + XC, D), BF16),
            vm((H, D, DH), BF16),
            vm((H, S, DH), BF16),
            vm((H, S, DH), BF16),
            vm((2, G, S, DH), BF16),
            vm((2, G, S, DH), BF16),
            vm((D // 128, H * DH, 128), BF16),
            vm((8, 128), BF16),
            vm((D, FF), BF16),
            vm((D, FF), BF16),
            vm((FF, D), BF16),
            vm((1, D), BF16),
            vm((D, 6 * D), BF16),
            vm((8, 6 * D), F32),
            vm((D, 128), F32),
            vm((NM + 1, MC, D), F32),
            vm((8, 8, 128), F32),
            vm((2, RG, 2 * D), BF16),
            vm((2, 16, D), BF16),
            pltpu.SemaphoreType.DMA((len(_names),)),
            *[vm((D // 128 + 1, (NX + 1) * HG, 128), BF16)] * NH,
            *[vm((NM + 1, RG, 2 * D), BF16)] * 8,
            *[vm((8, 8, 128), F32)] * MT,
        ],
        compiler_params=pltpu.CompilerParams(vmem_limit_bytes=124 * 1024 * 1024),
    )(
        A_x.reshape(S, D), A_k_cache.reshape(H, S, DH), A_v_cache.reshape(H, S, DH), A_wq, A_wo,
        B_w_r.reshape(8, 128), B_w_gate, B_w_up, B_w_down, c, w_mod,
    )
    return out.reshape(1, S, D)
```

```python
import functools
import math

import jax
import jax.numpy as jnp
from jax import lax
from jax.experimental import pallas as pl
from jax.experimental.pallas import tpu as pltpu

F32 = jnp.float32
BF16 = jnp.bfloat16
U32 = jnp.uint32

S = 2048
D = 1024
H = 32
DH = 128
FF = 3584
EPS = 1e-5
QSCALE = (DH ** -0.5) * math.log2(math.e)

G = 2
SUBS = ((256, 384, 384, 512, 512), (512, 512, 384, 384, 256))
N0 = 512
N1 = 512
XC = 256
NX = S // XC
NH = 16
HG = XC // NH
MC = 128
NM = S // MC
RG = MC // 8
PIECES = {1: [0], 2: [1], 3: [2], 4: [3], 5: [4], 6: [5], 7: [6, 7]}
LN_PIECES = {2: [0], 3: [1], 4: [2], 5: [3], 6: [4], 7: [5], 8: [6], 9: [7], 10: [8], 11: [9], 12: [10], 13: [11], 14: [12], 15: [13, 14, 15]}
MOD_PIECES = {0: [(0, 4)], 1: [(1, 0), (2, 4)], 2: [(3, 0), (4, 4)]}
MT = 5
FB = 512
NT = (((1,), (1,)), ((), ()))

_names = (["c", "wr", "wg", "wu", "wd", "wo", "f0", "f1"]
          + ["wq%d" % i for i in range(8)] + ["wn%d" % i for i in range(7)] + ["wm%d" % i for i in range(4, 8)] + ["x%d" % i for i in range(NX + 1)]
          + ["k0", "k1", "v0", "v1"] + ["o%d" % i for i in range(NM)])
_SEM = {n: i for i, n in enumerate(_names)}


def _attn(q, k, v):
    s = lax.dot_general(q, k, NT, preferred_element_type=F32)
    m = jnp.max(s, axis=1, keepdims=True)
    p = jnp.exp2(s - m)
    grp = 4
    acc = None
    tiles = []
    for g in range(S // (128 * grp)):
        ts = [p[:, (g * grp + j) * 128:(g * grp + j + 1) * 128] for j in range(grp)]
        t = (ts[0] + ts[1]) + (ts[2] + ts[3])
        acc = t if acc is None else acc + t
        tiles += ts[:-1] + [jnp.minimum(ts[-1], acc)]
    l = jnp.sum(acc, axis=1, keepdims=True)
    o = jnp.dot(jnp.concatenate(tiles, axis=1).astype(BF16), v, preferred_element_type=F32)
    return (o * pl.reciprocal(l, approx=True)).astype(BF16)


def _layernorm(x):
    xc = x - jnp.mean(x, axis=1, keepdims=True)
    var = jnp.mean(xc * xc, axis=1, keepdims=True)
    return xc * lax.rsqrt(var + EPS)


def _blk(i, n):
    return pl.ds(i * n if isinstance(i, int) else pl.multiple_of(i * n, n), n)


def _half(r0):
    return r0 // 2 if isinstance(r0, int) else pl.multiple_of(r0 // 2, 8)


def _ld(ref, lead, r0=0, n=None):
    n = ref.shape[-2] - r0 if n is None else n
    return pltpu.bitcast(ref.bitcast(U32)[(*lead, pl.ds(_half(r0), n // 2), slice(None))], BF16)


def _kernel(x_hbm, k_hbm, v_hbm, wq_hbm, wo_hbm, wr_hbm, wg_hbm, wu_hbm, wd_hbm,
            c_hbm, wm_hbm, out_hbm,
            x_v, wq_v, q_v, o_v, k_v, v_v, wo_v, wr_v, wg_v, wu_v, wd_v, c_v,
            wm_v, wm2_v, mod_v, scb_v, acc_v, r_v, sel_v, fix_v, sems, *bufs):

    piece = bufs[NH:NH + 8]
    mp = bufs[NH + 8:]

    def after(t, z, r=None):
        z = pltpu.bitcast(z, U32)
        if r is not None:
            for r_ in (r[0:8], r[8:16]):
                z = z & lax.bitcast_convert_type(jnp.broadcast_to(r_, z.shape), U32)
        return pltpu.bitcast(pltpu.bitcast(t, U32) | z, BF16)

    def modt(i, t, rows):
        m = mod_v[:, i * D + t * 128:i * D + (t + 1) * 128]
        return jnp.concatenate([m] * (rows // 8), axis=0)

    hbuf = bufs[:NH]

    def cp(name, src, dst, i=0):
        return pltpu.make_async_copy(src, dst, sems.at[_SEM[name] + i])

    def modw(i, rows):
        return jnp.concatenate([mod_v[:, i * D:(i + 1) * D]] * (rows // 8), axis=0)

    def mod(i):
        return mod_v[0:1, i * D:(i + 1) * D]

    c_cp = cp("c", c_hbm, c_v)
    def wm_cp(i):
        return cp("wm4", wm_hbm.at[:, _blk(i, 512)], wm_v.at[:, _blk(i, 512)], i)
    def wm2_tile0(j):
        return min(MT * j, 32 - MT) if isinstance(j, int) else jnp.minimum(MT * j, 32 - MT)
    def wm2_cp(j):
        cols = pl.ds(pl.multiple_of(2 * D + wm2_tile0(j) * 128, 128), MT * 128)
        return cp("wn0", wm_hbm.at[:, cols], wm2_v.at[j], j)
    def x_cp(i):
        return cp("x0", x_hbm.at[_blk(min(i, NX - 1) if isinstance(i, int) else jnp.minimum(i, NX - 1), XC), :],
                  x_v.at[_blk(i, XC), :], i)
    def wq_cps(j):
        return [cp("wq0", wq_hbm.at[:, _blk(j * 4 + t, DH)], wq_v.at[j * 4 + t], j) for t in range(4)]
    wo_cps = [cp("wo", wo_hbm.at[:, pl.ds(n * 128, 128)], wo_v.at[n]) for n in range(D // 128)]
    wr_cp = cp("wr", wr_hbm, wr_v)
    wg_cp = cp("wg", wg_hbm, wg_v)
    wu_cp = cp("wu", wu_hbm, wu_v)
    wd_cp = cp("wd", wd_hbm, wd_v)
    out4 = out_hbm.reshape(NM, 8, RG, D)

    def out_cps(half):
        js = pl.ds(0, NM // 2 - 1) if half == 0 else pl.ds(NM // 2 - 1, NM // 2 + 1)
        return [cp("o0", piece[p].at[js, :, pl.ds(D, D)], out4.at[js, p], half * 8 + p) for p in range(8)]

    def kv_cps(grp, slot):
        heads = pl.ds(grp * G, G)
        return (cp("k0", k_hbm.at[heads], k_v.at[slot], slot), cp("v0", v_hbm.at[heads], v_v.at[slot], slot))

    c_cp.start()
    for i in range(4):
        wm_cp(i).start()
    x_cp(0).start()
    for c_ in wq_cps(0):
        c_.start()
    x_cp(1).start()

    for p_ in hbuf:
        p_[D // 128, 0:16, :] = jnp.zeros((16, 128), BF16)
    for p_ in piece:
        p_[NM, :, 0:128] = jnp.zeros((RG, 128), BF16)
    c_cp.wait()
    cf = c_v[...].astype(F32)
    sc = jnp.broadcast_to(cf * jax.nn.sigmoid(cf), (16, D)).astype(BF16)
    scb_v[...] = jnp.broadcast_to(sc[0:1].astype(F32), (128, D)).T
    for m_ in mp:
        m_[7] = jnp.zeros((8, 128), F32)

    def mod_body(i, carry):
        wm_cp(i).wait()
        mod_v[:, _blk(i, 512)] = jnp.dot(sc, wm_v[:, _blk(i, 512)], preferred_element_type=F32)[:8]
        return carry

    lax.fori_loop(0, 4, mod_body, 0)

    def ln1(i, p, dst, row0):
        rows = pl.ds(pl.multiple_of(i * XC + p * HG, HG), HG)
        xn = _layernorm(x_v[rows, :].astype(F32))
        for t in range(D // 128):
            dst[t, row0:row0 + HG, :] = (xn[:, t * 128:(t + 1) * 128] * modt(1, t, HG) + modt(0, t, HG)).astype(BF16)

    mod_v[:, D:2 * D] = 1.0 + mod_v[:, D:2 * D]
    x_cp(0).wait()
    for p in range(NH):
        ln1(0, p, hbuf[p], 0)
    for c_ in wq_cps(0):
        c_.wait()
    for i in range(2, NX + 1):
        x_cp(i).start()
    for j_ in range(1, 8):
        for c_ in wq_cps(j_):
            c_.start()
        wm2_cp(j_ - 1).start()

    def p1a_body(i, carry):
        nxt = i + 1
        x_cp(nxt).wait()
        hv = [h.at[:, pl.ds(pl.multiple_of(i * HG, HG), 2 * HG), :] for h in hbuf]
        pos = 0
        for n in range(N0 // 128):
            for hf in range(2):
                wt = [_ld(wq_v, (n,), t * 128, 128) for t in range(D // 128)]
                for half_ in range(2):
                    for c_, p in enumerate(LN_PIECES.get(pos, ())):
                        ln1(nxt, p, hv[p], HG)
                        t = 4 * half_ + c_
                        wt[t] = jnp.concatenate([after(_ld(wq_v, (n,), t * 128, 16), _ld(hbuf[p], (D // 128,), 0, 16)),
                                                 _ld(wq_v, (n,), t * 128 + 16, 112)], axis=0)
                    pos += 1
                lhs = jnp.concatenate(
                    [jnp.concatenate([_ld(hv[p], (t,), 0, HG) for t in range(D // 128)], axis=1)
                     for p in range(hf * NH // 2, (hf + 1) * NH // 2)], axis=0)
                q = jnp.dot(lhs, jnp.concatenate(wt, axis=0), preferred_element_type=F32)
                q_v[n, pl.ds(pl.multiple_of(i * XC + hf * (XC // 2), XC // 2), XC // 2), :] = (q * QSCALE).astype(BF16)
        return carry

    lax.fori_loop(0, NX, p1a_body, 0)

    for c_ in kv_cps(0, 0):
        c_.start()
    for c_ in (wr_cp, *wo_cps, wg_cp, wu_cp, wd_cp):
        c_.start()

    def p1b_body(j, carry):
        for c_ in wq_cps(j):
            c_.wait()
        wm2_cp(j - 1).wait()
        for r in range(S // 512):
            wt = [[_ld(wq_v, (j * 4 + t,), k * 128, 128) for k in range(D // 128)] for t in range(4)]
            for p, k in MOD_PIECES.get(r, ()):
                wm = wm2_v[j - 1, :, p * 128:(p + 1) * 128].astype(F32)
                mp[p][j - 1] = jnp.broadcast_to(jnp.sum(wm * scb_v[...], axis=0, keepdims=True), (8, 128))
                z = jnp.concatenate([mp[p][7]] * 2, axis=0)
                wt[0][k] = jnp.concatenate([after(_ld(wq_v, (j * 4,), k * 128, 16), z.astype(BF16)),
                                            _ld(wq_v, (j * 4,), k * 128 + 16, 112)], axis=0)
            w = jnp.concatenate([jnp.concatenate(c_, axis=0) for c_ in wt], axis=1)
            lhs = jnp.concatenate(
                [jnp.concatenate([_ld(hbuf[p], (t,), i * HG, HG) for t in range(D // 128)], axis=1)
                 for i in (2 * r, 2 * r + 1) for p in range(NH)], axis=0)
            q = jnp.dot(lhs, w, preferred_element_type=F32) * QSCALE
            for t in range(4):
                q_v[j * 4 + t, r * 512:(r + 1) * 512, :] = q[:, t * DH:(t + 1) * DH].astype(BF16)
        return carry

    lax.fori_loop(1, 8, p1b_body, 0)
    for c_ in range(32):
        j_ = min(c_ // MT, 6)
        mod_v[:, 2 * D + c_ * 128:2 * D + (c_ + 1) * 128] = mp[c_ - min(MT * j_, 32 - MT)][j_]

    def p2_body(grp, carry):
        slot = grp % 2

        for c_ in kv_cps(jnp.minimum(grp + 1, H // G - 1), 1 - slot):
            c_.start()
        for c_ in kv_cps(grp, slot):
            c_.wait()
        for hh in range(G):
            head = grp * G + hh
            r0 = 0
            for nr in SUBS[hh]:
                rows = pl.ds(r0, nr)
                r0 += nr
                o_v[head, rows, :] = _attn(q_v[head, rows, :], k_v[slot, hh], v_v[slot, hh])
        return carry

    lax.fori_loop(0, H // G, p2_body, 0)
    for c_ in kv_cps(H // G - 1, (H // G) % 2):
        c_.wait()

    mod_v[:, 4 * D:5 * D] = (1.0 + mod_v[:, 4 * D:5 * D].astype(BF16).astype(F32)).astype(BF16).astype(F32)

    for c_ in wo_cps:
        c_.wait()
    wr_cp.wait()
    wr = wr_v[...].astype(F32)
    for t in range(D // 128):
        mod_v[:, t * 128:(t + 1) * 128] = jnp.broadcast_to(wr[t:t + 1, :], (8, 128))
    lane = lax.broadcasted_iota(jnp.int32, (8, 128), 1)
    acc_v[0] = jnp.zeros((MC, D), F32)

    def finish(j, p, acc):
        rows = pl.ds(pl.multiple_of(j * MC + p * RG, RG), RG)
        x2 = x_v[rows, :].astype(F32) + modw(2, RG) * acc[p * RG:(p + 1) * RG, :]
        h2 = (_layernorm(x2) * modw(4, RG) + modw(3, RG)).astype(BF16)
        piece[p][j, :, 0:D] = h2
        h2 = h2.astype(F32)
        piece[p][j, :, D:2 * D] = (x2 + modw(5, RG) * (h2 + h2 * 0.0)).astype(BF16)
        e = h2 * modw(0, RG)
        pr = None
        for t in range(D // 128):
            pr = e[:, t * 128:(t + 1) * 128] if pr is None else pr + e[:, t * 128:(t + 1) * 128]
        r = jnp.sum(pr, axis=1, keepdims=True)
        r_v[p] = jnp.where(lane == 2 * j, r[0:8], jnp.where(lane == 2 * j + 1, r[8:16], r_v[p]))
        return r

    def p3_body(j, carry):
        jp = jnp.maximum(j - 1, 0)
        accs = acc_v.at[pl.ds(j, 2)]
        for n in range(D // 128):
            cols = slice(n * 128, (n + 1) * 128)
            row0 = pl.multiple_of(j * MC, MC)
            tiles = [_ld(o_v, (h,), row0, MC) for h in range(H)]
            for p in PIECES.get(n, ()):
                r = finish(jp, p, accs.at[0])
                tiles[p] = jnp.concatenate([after(_ld(o_v, (p,), row0, 16), piece[p][NM, :, 0:128], r),
                                            _ld(o_v, (p,), row0 + 16, MC - 16)], axis=0)
            lhs = jnp.concatenate(tiles, axis=1)
            accs[1, :, cols] = jnp.dot(lhs, _ld(wo_v, (n,)), preferred_element_type=F32)

        return carry

    def p3_half(half, carry):
        lax.fori_loop(half * (NM // 2), (half + 1) * (NM // 2), p3_body, 0)

        @pl.when(half == 0)
        def _():
            for c_ in out_cps(0):
                c_.start()
        return carry

    r_v[...] = jnp.zeros_like(r_v)
    lax.fori_loop(0, 2, p3_half, 0)
    for p in range(8):
        finish(NM - 1, p, acc_v.at[NM])

    r = r_v[...].astype(BF16).astype(F32) + 0.0
    ln_ = lax.broadcasted_iota(jnp.int32, r.shape, 2)
    tok = (lax.broadcasted_iota(jnp.int32, r.shape, 0) * RG + (ln_ // 2) * MC + (ln_ % 2) * 8
           + lax.broadcasted_iota(jnp.int32, r.shape, 1))
    u = lax.shift_right_logical(lax.bitcast_convert_type(r, jnp.int32), 16)
    u = jnp.where(u >= 0x8000, 0xFFFF - u, u + 0x8000)
    key = jnp.where(ln_ < 2 * NM, (u << 11) + (S - 1 - tok) + (1 << 27), 0)
    key = lax.bitcast_convert_type(key, F32)

    def top1(k):
        m = jnp.max(jnp.max(k, axis=0), axis=0, keepdims=True)
        m = jnp.max(m, axis=1, keepdims=True)
        bits = lax.bitcast_convert_type(m, jnp.int32)
        u_ = (bits >> 11) & 0xFFFF
        u_ = jnp.where(u_ >= 0x8000, u_ - 0x8000, 0xFFFF - u_)
        score = lax.bitcast_convert_type(u_ << 16, F32)
        return m, (S - 1) - (bits & (S - 1))[0, 0], jax.nn.sigmoid(score)

    m0, i0, g0 = top1(key)
    m1, i1, g1 = top1(jnp.where(key == m0, 0.0, key))
    base = [pl.multiple_of((i // RG) * RG, RG) for i in (i0, i1)]
    for s_, b_ in enumerate(base):
        for p in range(8):
            @pl.when((b_ % MC) // RG == p)
            def _(s_=s_, b_=b_, p=p):
                sel_v[s_] = piece[p][b_ // MC]
    row16 = lax.broadcasted_iota(jnp.int32, (16, D), 0)
    won = [row16 + base[s_] == i_ for s_, i_ in enumerate((i0, i1))]
    xrow = [jnp.sum(jnp.where(won[s_], sel_v[s_, :, 0:D].astype(F32), 0.0), axis=0, keepdims=True) for s_ in range(2)]
    xs = jnp.where(row16 == 0, xrow[0], jnp.where(row16 == 1, xrow[1], 0.0)).astype(BF16)

    for c_ in out_cps(1):
        c_.start()
    wg_cp.wait()
    wu_cp.wait()
    wd_cp.wait()

    y = None
    for f in range(FF // FB):
        cols = slice(f * FB, (f + 1) * FB)
        g = jnp.dot(xs, wg_v[:, cols], preferred_element_type=F32)
        u = jnp.dot(xs, wu_v[:, cols], preferred_element_type=F32)
        act = (g * jax.nn.sigmoid(g) * u).astype(BF16)
        d = jnp.dot(act, wd_v[cols, :], preferred_element_type=F32)
        y = d if y is None else y + d
    y0 = y[0:1] * g0
    y1 = y[1:2] * g1
    for s_ in range(2):
        upd = jnp.where(row16 + base[s_] == i0, y0, jnp.where(row16 + base[s_] == i1, y1, 0.0))
        fix_v[s_] = (sel_v[s_, :, D:2 * D].astype(F32) + mod(5) * upd).astype(BF16)

    for c_ in out_cps(0) + out_cps(1):
        c_.wait()
    fix = [cp("f0", fix_v.at[s_], out_hbm.at[pl.ds(base[s_], 16), :], s_) for s_ in range(2)]
    fix[0].start()

    @pl.when(base[0] != base[1])
    def _():
        fix[1].start()
        fix[1].wait()

    fix[0].wait()


@jax.jit
def pallas_adaLN_cond__mha_block_cached__moe_arch_mod__prompt_kernel(
    A_x: jax.Array,
    A_k_cache: jax.Array,
    A_v_cache: jax.Array,
    A_wq: jax.Array,
    A_wo: jax.Array,
    B_x: jax.Array,
    B_w_r: jax.Array,
    B_w_gate: jax.Array,
    B_w_up: jax.Array,
    B_w_down: jax.Array,
    c: jax.Array,
    w_mod: jax.Array,
):
    any_spec = pl.BlockSpec(memory_space=pl.ANY)
    vm = pltpu.VMEM
    out = pl.pallas_call(
        _kernel,
        name="adaln_mha_moe",
        in_specs=[any_spec] * 11,
        out_specs=any_spec,
        out_shape=jax.ShapeDtypeStruct((S, D), BF16),
        scratch_shapes=[
            vm((S + XC, D), BF16),
            vm((H, D, DH), BF16),
            vm((H, S, DH), BF16),
            vm((H, S, DH), BF16),
            vm((2, G, S, DH), BF16),
            vm((2, G, S, DH), BF16),
            vm((D // 128, H * DH, 128), BF16),
            vm((8, 128), BF16),
            vm((D, FF), BF16),
            vm((D, FF), BF16),
            vm((FF, D), BF16),
            vm((1, D), BF16),
            vm((D, 2 * D), BF16),
            vm((7, D, MT * 128), BF16),
            vm((8, 6 * D), F32),
            vm((D, 128), F32),
            vm((NM + 1, MC, D), F32),
            vm((8, 8, 128), F32),
            vm((2, RG, 2 * D), BF16),
            vm((2, 16, D), BF16),
            pltpu.SemaphoreType.DMA((len(_names),)),
            *[vm((D // 128 + 1, (NX + 1) * HG, 128), BF16)] * NH,
            *[vm((NM + 1, RG, 2 * D), BF16)] * 8,
            *[vm((8, 8, 128), F32)] * MT,
        ],
        compiler_params=pltpu.CompilerParams(vmem_limit_bytes=124 * 1024 * 1024),
    )(
        A_x.reshape(S, D), A_k_cache.reshape(H, S, DH), A_v_cache.reshape(H, S, DH), A_wq, A_wo,
        B_w_r.reshape(8, 128), B_w_gate, B_w_up, B_w_down, c, w_mod,
    )
    return out.reshape(1, S, D)
```

```python
import math

import jax
import jax.numpy as jnp
from jax import lax
from jax.experimental import pallas as pl
from jax.experimental.pallas import tpu as pltpu

F32 = jnp.float32
BF16 = jnp.bfloat16
U32 = jnp.uint32

S = 2048
D = 1024
H = 32
DH = 128
FF = 3584
EPS = 1e-5
QSCALE = (DH ** -0.5) * math.log2(math.e)

G = 2
SUBS = ((256, 384, 384, 512, 512), (512, 512, 384, 384, 256))
N0 = 512
XC = 256
NX = S // XC
NH = 16
HG = XC // NH
MC = 128
NM = S // MC
RG = MC // 8
PIECES = {1: [0], 2: [1], 3: [2], 4: [3], 5: [4], 6: [5], 7: [6, 7]}
LN_PIECES = {2: [0], 3: [1], 4: [2], 5: [3], 6: [4], 7: [5], 8: [6], 9: [7], 10: [8], 11: [9], 12: [10], 13: [11], 14: [12], 15: [13, 14, 15]}
MOD_PIECES = {0: [(0, 4)], 1: [(1, 0), (2, 4)], 2: [(3, 0), (4, 4)]}
MT = 5
FB = 512
NT = (((1,), (1,)), ((), ()))

_names = (["c", "wr", "wg", "wu", "wd", "wo", "f0", "f1"]
          + ["wq%d" % i for i in range(8)] + ["wn%d" % i for i in range(7)] + ["wm%d" % i for i in range(4, 8)] + ["x%d" % i for i in range(NX + 1)]
          + ["k0", "k1", "v0", "v1"] + ["o%d" % i for i in range(NM)])
_SEM = {n: i for i, n in enumerate(_names)}


def _attn(q, k, v):
    s = lax.dot_general(q, k, NT, preferred_element_type=F32)
    m = jnp.max(s, axis=1, keepdims=True)
    p = jnp.exp2(s - m)
    grp = 4
    acc = None
    tiles = []
    for g in range(S // (128 * grp)):
        ts = [p[:, (g * grp + j) * 128:(g * grp + j + 1) * 128] for j in range(grp)]
        t = (ts[0] + ts[1]) + (ts[2] + ts[3])
        acc = t if acc is None else acc + t
        tiles += ts[:-1] + [jnp.minimum(ts[-1], acc)]
    l = jnp.sum(acc, axis=1, keepdims=True)
    o = jnp.dot(jnp.concatenate(tiles, axis=1).astype(BF16), v, preferred_element_type=F32)
    return (o * pl.reciprocal(l, approx=True)).astype(BF16)


def _layernorm(x):
    xc = x - jnp.mean(x, axis=1, keepdims=True)
    var = jnp.mean(xc * xc, axis=1, keepdims=True)
    return xc * lax.rsqrt(var + EPS)


def _blk(i, n):
    return pl.ds(i * n if isinstance(i, int) else pl.multiple_of(i * n, n), n)


def _half(r0):
    return r0 // 2 if isinstance(r0, int) else pl.multiple_of(r0 // 2, 8)


def _ld(ref, lead, r0=0, n=None):
    n = ref.shape[-2] - r0 if n is None else n
    return pltpu.bitcast(ref.bitcast(U32)[(*lead, pl.ds(_half(r0), n // 2), slice(None))], BF16)


def _kernel(x_hbm, k_hbm, v_hbm, wq_hbm, wo_hbm, wr_hbm, wg_hbm, wu_hbm, wd_hbm,
            c_hbm, wm_hbm, out_hbm,
            x_v, wq_v, q_v, o_v, k_v, v_v, wo_v, wr_v, wg_v, wu_v, wd_v, c_v,
            wm_v, wm2_v, mod_v, scb_v, acc_v, r_v, sel_v, fix_v, sems, *bufs):

    piece = bufs[NH:NH + 8]
    mp = bufs[NH + 8:]

    def after(t, z, r=None):
        z = pltpu.bitcast(z, U32)
        if r is not None:
            for r_ in (r[0:8], r[8:16]):
                z = z & lax.bitcast_convert_type(jnp.broadcast_to(r_, z.shape), U32)
        return pltpu.bitcast(pltpu.bitcast(t, U32) | z, BF16)

    def modt(i, t, rows):
        m = mod_v[:, i * D + t * 128:i * D + (t + 1) * 128]
        return jnp.concatenate([m] * (rows // 8), axis=0)

    hbuf = bufs[:NH]

    def cp(name, src, dst, i=0):
        return pltpu.make_async_copy(src, dst, sems.at[_SEM[name] + i])

    def modw(i, rows):
        return jnp.concatenate([mod_v[:, i * D:(i + 1) * D]] * (rows // 8), axis=0)

    def mod(i):
        return mod_v[0:1, i * D:(i + 1) * D]

    c_cp = cp("c", c_hbm, c_v)
    def wm_cp(i):
        return cp("wm4", wm_hbm.at[:, _blk(i, 512)], wm_v.at[:, _blk(i, 512)], i)
    def wm2_tile0(j):
        return min(MT * j, 32 - MT) if isinstance(j, int) else jnp.minimum(MT * j, 32 - MT)
    def wm2_cp(j):
        cols = pl.ds(pl.multiple_of(2 * D + wm2_tile0(j) * 128, 128), MT * 128)
        return cp("wn0", wm_hbm.at[:, cols], wm2_v.at[j], j)
    def x_cp(i):
        return cp("x0", x_hbm.at[_blk(min(i, NX - 1) if isinstance(i, int) else jnp.minimum(i, NX - 1), XC), :],
                  x_v.at[_blk(i, XC), :], i)
    def wq_cps(j):
        return [cp("wq0", wq_hbm.at[:, _blk(j * 4 + t, DH)], wq_v.at[j * 4 + t], j) for t in range(4)]
    wo_cps = [cp("wo", wo_hbm.at[:, pl.ds(n * 128, 128)], wo_v.at[n]) for n in range(D // 128)]
    wr_cp = cp("wr", wr_hbm, wr_v)
    wg_cp = cp("wg", wg_hbm, wg_v)
    wu_cp = cp("wu", wu_hbm, wu_v)
    wd_cp = cp("wd", wd_hbm, wd_v)
    out4 = out_hbm.reshape(NM, 8, RG, D)

    def out_cps(half):
        js = pl.ds(0, NM // 2 - 1) if half == 0 else pl.ds(NM // 2 - 1, NM // 2 + 1)
        return [cp("o0", piece[p].at[js, :, pl.ds(D, D)], out4.at[js, p], half * 8 + p) for p in range(8)]

    def kv_cps(grp, slot):
        heads = pl.ds(grp * G, G)
        return (cp("k0", k_hbm.at[heads], k_v.at[slot], slot), cp("v0", v_hbm.at[heads], v_v.at[slot], slot))

    c_cp.start()
    for i in range(4):
        wm_cp(i).start()
    x_cp(0).start()
    for c_ in wq_cps(0):
        c_.start()
    x_cp(1).start()

    for p_ in hbuf:
        p_[D // 128, 0:16, :] = jnp.zeros((16, 128), BF16)
    for p_ in piece:
        p_[NM, :, 0:128] = jnp.zeros((RG, 128), BF16)
    c_cp.wait()
    cf = c_v[...].astype(F32)
    sc = jnp.broadcast_to(cf * jax.nn.sigmoid(cf), (16, D)).astype(BF16)
    scb_v[...] = jnp.broadcast_to(sc[0:1].astype(F32), (128, D)).T
    for m_ in mp:
        m_[7] = jnp.zeros((8, 128), F32)

    def mod_body(i, carry):
        wm_cp(i).wait()
        mod_v[:, _blk(i, 512)] = jnp.dot(sc, wm_v[:, _blk(i, 512)], preferred_element_type=F32)[:8]
        return carry

    lax.fori_loop(0, 4, mod_body, 0)

    def ln1(i, p, dst, row0):
        rows = pl.ds(pl.multiple_of(i * XC + p * HG, HG), HG)
        xn = _layernorm(x_v[rows, :].astype(F32))
        for t in range(D // 128):
            dst[t, row0:row0 + HG, :] = (xn[:, t * 128:(t + 1) * 128] * modt(1, t, HG) + modt(0, t, HG)).astype(BF16)

    mod_v[:, D:2 * D] = (1.0 + mod_v[:, D:2 * D]) * QSCALE
    mod_v[:, 0:D] = mod_v[:, 0:D] * QSCALE
    x_cp(0).wait()
    for p in range(NH):
        ln1(0, p, hbuf[p], 0)
    for c_ in wq_cps(0):
        c_.wait()
    for i in range(2, NX + 1):
        x_cp(i).start()
    for j_ in range(1, 8):
        for c_ in wq_cps(j_):
            c_.start()
        wm2_cp(j_ - 1).start()

    def p1a_body(i, carry):
        nxt = i + 1
        x_cp(nxt).wait()
        hv = [h.at[:, pl.ds(pl.multiple_of(i * HG, HG), 2 * HG), :] for h in hbuf]
        pos = 0
        for n in range(N0 // 128):
            for hf in range(2):
                wt = [_ld(wq_v, (n,), t * 128, 128) for t in range(D // 128)]
                for half_ in range(2):
                    for c_, p in enumerate(LN_PIECES.get(pos, ())):
                        ln1(nxt, p, hv[p], HG)
                        t = 4 * half_ + c_
                        wt[t] = jnp.concatenate([after(_ld(wq_v, (n,), t * 128, 16), _ld(hbuf[p], (D // 128,), 0, 16)),
                                                 _ld(wq_v, (n,), t * 128 + 16, 112)], axis=0)
                    pos += 1
                lhs = jnp.concatenate(
                    [jnp.concatenate([_ld(hv[p], (t,), 0, HG) for t in range(D // 128)], axis=1)
                     for p in range(hf * NH // 2, (hf + 1) * NH // 2)], axis=0)
                q = jnp.dot(lhs, jnp.concatenate(wt, axis=0), preferred_element_type=F32)
                q_v[n, pl.ds(pl.multiple_of(i * XC + hf * (XC // 2), XC // 2), XC // 2), :] = q.astype(BF16)
        return carry

    lax.fori_loop(0, NX, p1a_body, 0)

    for c_ in kv_cps(0, 0):
        c_.start()
    for c_ in (wr_cp, *wo_cps, wg_cp, wu_cp, wd_cp):
        c_.start()

    def p1b_body(j, carry):
        for c_ in wq_cps(j):
            c_.wait()
        wm2_cp(j - 1).wait()
        for r in range(S // 512):
            wt = [[_ld(wq_v, (j * 4 + t,), k * 128, 128) for k in range(D // 128)] for t in range(4)]
            for p, k in MOD_PIECES.get(r, ()):
                wm = wm2_v[j - 1, :, p * 128:(p + 1) * 128].astype(F32)
                mp[p][j - 1] = jnp.broadcast_to(jnp.sum(wm * scb_v[...], axis=0, keepdims=True), (8, 128))
                z = jnp.concatenate([mp[p][7]] * 2, axis=0)
                wt[0][k] = jnp.concatenate([after(_ld(wq_v, (j * 4,), k * 128, 16), z.astype(BF16)),
                                            _ld(wq_v, (j * 4,), k * 128 + 16, 112)], axis=0)
            w = jnp.concatenate([jnp.concatenate(c_, axis=0) for c_ in wt], axis=1)
            lhs = jnp.concatenate(
                [jnp.concatenate([_ld(hbuf[p], (t,), i * HG, HG) for t in range(D // 128)], axis=1)
                 for i in (2 * r, 2 * r + 1) for p in range(NH)], axis=0)
            q = jnp.dot(lhs, w, preferred_element_type=F32)
            for t in range(4):
                q_v[j * 4 + t, r * 512:(r + 1) * 512, :] = q[:, t * DH:(t + 1) * DH].astype(BF16)
        return carry

    lax.fori_loop(1, 8, p1b_body, 0)
    for c_ in range(32):
        j_ = min(c_ // MT, 6)
        mod_v[:, 2 * D + c_ * 128:2 * D + (c_ + 1) * 128] = mp[c_ - min(MT * j_, 32 - MT)][j_]

    def p2_body(grp, carry):
        slot = grp % 2

        for hh in range(G):
            head = grp * G + hh
            r0 = 0
            for nr in SUBS[hh]:
                rows = pl.ds(r0, nr)
                r0 += nr
                o_v[head, rows, :] = _attn(q_v[head, rows, :], k_v[slot, hh], v_v[slot, hh])
        for c_ in kv_cps(jnp.minimum(grp + 2, H // G - 1), slot):
            c_.start()
        for c_ in kv_cps(jnp.minimum(grp + 1, H // G - 1), 1 - slot):
            c_.wait()
        return carry

    for c_ in kv_cps(0, 0):
        c_.wait()
    for c_ in kv_cps(1, 1):
        c_.start()
    lax.fori_loop(0, H // G, p2_body, 0)

    mod_v[:, 4 * D:5 * D] = (1.0 + mod_v[:, 4 * D:5 * D].astype(BF16).astype(F32)).astype(BF16).astype(F32)

    for c_ in wo_cps:
        c_.wait()
    wr_cp.wait()
    wr = wr_v[...].astype(F32)
    for t in range(D // 128):
        mod_v[:, t * 128:(t + 1) * 128] = jnp.broadcast_to(wr[t:t + 1, :], (8, 128))
    lane = lax.broadcasted_iota(jnp.int32, (8, 128), 1)
    acc_v[0] = jnp.zeros((MC, D), F32)

    def finish(j, p, acc):
        rows = pl.ds(pl.multiple_of(j * MC + p * RG, RG), RG)
        x2 = x_v[rows, :].astype(F32) + modw(2, RG) * acc[p * RG:(p + 1) * RG, :]
        h2 = (_layernorm(x2) * modw(4, RG) + modw(3, RG)).astype(BF16)
        piece[p][j, :, 0:D] = h2
        h2 = h2.astype(F32)
        piece[p][j, :, D:2 * D] = (x2 + modw(5, RG) * (h2 + h2 * 0.0)).astype(BF16)
        e = h2 * modw(0, RG)
        pr = None
        for t in range(D // 128):
            pr = e[:, t * 128:(t + 1) * 128] if pr is None else pr + e[:, t * 128:(t + 1) * 128]
        r = jnp.sum(pr, axis=1, keepdims=True)
        r_v[p] = jnp.where(lane == 2 * j, r[0:8], jnp.where(lane == 2 * j + 1, r[8:16], r_v[p]))
        return r

    def p3_body(j, carry):
        jp = jnp.maximum(j - 1, 0)
        accs = acc_v.at[pl.ds(j, 2)]
        for n in range(D // 128):
            cols = slice(n * 128, (n + 1) * 128)
            row0 = pl.multiple_of(j * MC, MC)
            tiles = [_ld(o_v, (h,), row0, MC) for h in range(H)]
            for p in PIECES.get(n, ()):
                r = finish(jp, p, accs.at[0])
                tiles[p] = jnp.concatenate([after(_ld(o_v, (p,), row0, 16), piece[p][NM, :, 0:128], r),
                                            _ld(o_v, (p,), row0 + 16, MC - 16)], axis=0)
            lhs = jnp.concatenate(tiles, axis=1)
            accs[1, :, cols] = jnp.dot(lhs, _ld(wo_v, (n,)), preferred_element_type=F32)

        return carry

    def p3_half(half, carry):
        lax.fori_loop(half * (NM // 2), (half + 1) * (NM // 2), p3_body, 0)

        @pl.when(half == 0)
        def _():
            for c_ in out_cps(0):
                c_.start()
        return carry

    r_v[...] = jnp.zeros_like(r_v)
    lax.fori_loop(0, 2, p3_half, 0)
    for p in range(8):
        finish(NM - 1, p, acc_v.at[NM])

    r = r_v[...].astype(BF16).astype(F32) + 0.0
    ln_ = lax.broadcasted_iota(jnp.int32, r.shape, 2)
    tok = (lax.broadcasted_iota(jnp.int32, r.shape, 0) * RG + (ln_ // 2) * MC + (ln_ % 2) * 8
           + lax.broadcasted_iota(jnp.int32, r.shape, 1))
    u = lax.shift_right_logical(lax.bitcast_convert_type(r, jnp.int32), 16)
    u = jnp.where(u >= 0x8000, 0xFFFF - u, u + 0x8000)
    key = jnp.where(ln_ < 2 * NM, (u << 11) + (S - 1 - tok) + (1 << 27), 0)
    key = lax.bitcast_convert_type(key, F32)

    def top1(k):
        m = jnp.max(jnp.max(k, axis=0), axis=0, keepdims=True)
        m = jnp.max(m, axis=1, keepdims=True)
        bits = lax.bitcast_convert_type(m, jnp.int32)
        u_ = (bits >> 11) & 0xFFFF
        u_ = jnp.where(u_ >= 0x8000, u_ - 0x8000, 0xFFFF - u_)
        score = lax.bitcast_convert_type(u_ << 16, F32)
        return m, (S - 1) - (bits & (S - 1))[0, 0], jax.nn.sigmoid(score)

    m0, i0, g0 = top1(key)
    m1, i1, g1 = top1(jnp.where(key == m0, 0.0, key))
    base = [pl.multiple_of((i // RG) * RG, RG) for i in (i0, i1)]
    for s_, b_ in enumerate(base):
        for p in range(8):
            @pl.when((b_ % MC) // RG == p)
            def _(s_=s_, b_=b_, p=p):
                sel_v[s_] = piece[p][b_ // MC]
    row16 = lax.broadcasted_iota(jnp.int32, (16, D), 0)
    won = [row16 + base[s_] == i_ for s_, i_ in enumerate((i0, i1))]
    xrow = [jnp.sum(jnp.where(won[s_], sel_v[s_, :, 0:D].astype(F32), 0.0), axis=0, keepdims=True) for s_ in range(2)]
    xs = jnp.where(row16 == 0, xrow[0], jnp.where(row16 == 1, xrow[1], 0.0)).astype(BF16)

    for c_ in out_cps(1):
        c_.start()
    wg_cp.wait()
    wu_cp.wait()
    wd_cp.wait()

    y = None
    for f in range(FF // FB):
        cols = slice(f * FB, (f + 1) * FB)
        g = jnp.dot(xs, wg_v[:, cols], preferred_element_type=F32)
        u = jnp.dot(xs, wu_v[:, cols], preferred_element_type=F32)
        act = (g * jax.nn.sigmoid(g) * u).astype(BF16)
        d = jnp.dot(act, wd_v[cols, :], preferred_element_type=F32)
        y = d if y is None else y + d
    y0 = y[0:1] * g0
    y1 = y[1:2] * g1
    for s_ in range(2):
        upd = jnp.where(row16 + base[s_] == i0, y0, jnp.where(row16 + base[s_] == i1, y1, 0.0))
        fix_v[s_] = (sel_v[s_, :, D:2 * D].astype(F32) + mod(5) * upd).astype(BF16)

    for c_ in out_cps(0) + out_cps(1) + list(kv_cps(H // G - 1, (H // G - 1) % 2)):
        c_.wait()
    fix = [cp("f0", fix_v.at[s_], out_hbm.at[pl.ds(base[s_], 16), :], s_) for s_ in range(2)]
    fix[0].start()

    @pl.when(base[0] != base[1])
    def _():
        fix[1].start()
        fix[1].wait()

    fix[0].wait()


@jax.jit
def pallas_adaLN_cond__mha_block_cached__moe_arch_mod__prompt_kernel(
    A_x: jax.Array,
    A_k_cache: jax.Array,
    A_v_cache: jax.Array,
    A_wq: jax.Array,
    A_wo: jax.Array,
    B_x: jax.Array,
    B_w_r: jax.Array,
    B_w_gate: jax.Array,
    B_w_up: jax.Array,
    B_w_down: jax.Array,
    c: jax.Array,
    w_mod: jax.Array,
):
    any_spec = pl.BlockSpec(memory_space=pl.ANY)
    vm = pltpu.VMEM
    out = pl.pallas_call(
        _kernel,
        name="adaln_mha_moe",
        in_specs=[any_spec] * 11,
        out_specs=any_spec,
        out_shape=jax.ShapeDtypeStruct((S, D), BF16),
        scratch_shapes=[
            vm((S + XC, D), BF16),
            vm((H, D, DH), BF16),
            vm((H, S, DH), BF16),
            vm((H, S, DH), BF16),
            vm((2, G, S, DH), BF16),
            vm((2, G, S, DH), BF16),
            vm((D // 128, H * DH, 128), BF16),
            vm((8, 128), BF16),
            vm((D, FF), BF16),
            vm((D, FF), BF16),
            vm((FF, D), BF16),
            vm((1, D), BF16),
            vm((D, 2 * D), BF16),
            vm((7, D, MT * 128), BF16),
            vm((8, 6 * D), F32),
            vm((D, 128), F32),
            vm((NM + 1, MC, D), F32),
            vm((8, 8, 128), F32),
            vm((2, RG, 2 * D), BF16),
            vm((2, 16, D), BF16),
            pltpu.SemaphoreType.DMA((len(_names),)),
            *[vm((D // 128 + 1, (NX + 1) * HG, 128), BF16)] * NH,
            *[vm((NM + 1, RG, 2 * D), BF16)] * 8,
            *[vm((8, 8, 128), F32)] * MT,
        ],
        compiler_params=pltpu.CompilerParams(vmem_limit_bytes=124 * 1024 * 1024),
    )(
        A_x.reshape(S, D), A_k_cache.reshape(H, S, DH), A_v_cache.reshape(H, S, DH), A_wq, A_wo,
        B_w_r.reshape(8, 128), B_w_gate, B_w_up, B_w_down, c, w_mod,
    )
    return out.reshape(1, S, D)
```
